```python
import jax
import jax.numpy as jnp

def _softmax(x, axis=-1):
    return jax.nn.softmax(x, axis=axis)
def _gelu(x):
    return jax.nn.gelu(x, approximate=True)
def _silu(x):
    return jax.nn.silu(x)
def _sigmoid(x):
    return jax.nn.sigmoid(x)
def _layernorm(x, axis=-1, eps=1e-5):
    m = jnp.mean(x, axis=axis, keepdims=True)
    v = jnp.var(x, axis=axis, keepdims=True)
    return (x - m) / jnp.sqrt(v + eps)
def _scatter_add(tgt, idx, src, axis=0):
    return tgt.at[idx].add(src)
def _segment_sum(src, seg, n):
    return jax.ops.segment_sum(src, seg, n)
class _Rng:
    def __init__(self, key):
        self._k = key
    def _next(self):
        self._k, sub = jax.random.split(self._k)
        return sub
    def normal(self, shape):
        return jax.random.normal(self._next(), shape, dtype=jnp.bfloat16)
    def randint(self, lo, hi, shape):
        return jax.random.randint(self._next(), shape, lo, hi, dtype=jnp.int32)
    def uniform(self, shape, lo=0.0, hi=1.0):
        return jax.random.uniform(self._next(), shape, jnp.bfloat16, lo, hi)
    def permutation(self, n):
        return jax.random.permutation(self._next(), n)


kernel_name = 'standalone__fused_io_aware_attn__prompt'

def setup_inputs():
    _rng = _Rng(jax.random.key(int.from_bytes(__import__("os").urandom(4), "little")))
    _w = (lambda a: (lambda t: t.astype(jnp.bfloat16) if jnp.issubdtype(t.dtype, jnp.floating) else t)(jnp.asarray(a)))
    B, H, S = 2, 32, 2048
    Dh = max(1, 1024 // 32)
    return {
        "q": _w((lambda *s: _rng.normal(s) * 0.05)(B, H, S, Dh)),
        "k": _w((lambda *s: _rng.normal(s) * 0.05)(B, H, S, Dh)),
        "v": _w((lambda *s: _rng.normal(s) * 0.05)(B, H, S, Dh)),
    }

def reference(q, k, v):
    scale = q.shape[-1] ** -0.5
    s = jnp.einsum('bhqd,bhkd->bhqk', q, k) * scale
    p = _softmax(s, axis=-1)
    return jnp.einsum('bhqk,bhkd->bhqd', p, v)
```

```python
import math

import jax
import jax.numpy as jnp
import jax.experimental.pallas as pl
import jax.experimental.pallas.tpu as pltpu

TQ = 512
TK = 128
LAG = 2
DELTA = 2


def _attn_kernel(q_ref, qn_ref, k0_ref, kn_ref, v_ref, o_ref,
                 s_ref, m_ref, m8_ref, kt_ref, flag_ref):
    D, S = q_ref.shape
    tq, tk = TQ, TK
    c = (D ** -0.5) * math.log2(math.e)
    t = pl.program_id(0)
    nq = S // tq
    nk = S // tk
    lead = nk + LAG
    ring = 2 * nk
    n_steps = nq * nk

    class QK:
        def __init__(self, qsrc, ksrc, m8, mfin):
            self.qsrc, self.ksrc, self.m8, self.mfin = qsrc, ksrc, m8, mfin
            self.qcache, self.ms = {}, {}

        def step(self, g):
            tile, j = divmod(g, nk)
            if tile not in self.qcache:
                ref, ti = self.qsrc(tile)
                x = ref[:, ti * tq:(ti + 1) * tq]
                self.qcache[tile] = (x.astype(jnp.float32) * c).astype(jnp.bfloat16)
            sl = pl.ds(j * tk, tk)
            ks = self.ksrc(tile)
            if ks is None:
                kc = kt_ref[sl, :]
            else:
                kc = ks[:, sl].T
                kt_ref[sl, :] = kc
            s = jnp.dot(kc, self.qcache[tile], preferred_element_type=jnp.float32)
            s_ref[pl.ds((g % ring) * tk, tk), :] = s
            ms = jnp.max(s.reshape(tk // 8, 8, tq), axis=0)
            self.ms[g] = ms
            self.m8 = ms if j == 0 else jnp.maximum(self.m8, ms)
            if j == nk - 1:
                self.mfin[tile] = jnp.broadcast_to(
                    jnp.max(self.m8, axis=0, keepdims=True), (8, tq))

    @pl.when(t == 0)
    def _():
        qk0 = QK(lambda tile: (q_ref, tile),
                 lambda tile: k0_ref if tile == 0 else None, None, {})
        for g in range(lead):
            qk0.step(g)
        m_ref[...] = qk0.mfin[0]
        m8_ref[...] = qk0.m8
        flag_ref[...] = jnp.ones(flag_ref.shape, flag_ref.dtype)

    flag = flag_ref[...] > 0
    qk = QK(lambda tile: (q_ref, tile) if tile < nq else (qn_ref, tile - nq),
            lambda tile: kn_ref if tile == nq else None,
            m8_ref[...], {0: m_ref[...]})
    l8 = acc = None
    for g in range(n_steps):
        tile, j = divmod(g, nk)
        qk.step(g + lead)
        s_cur = s_ref[pl.ds((g % ring) * tk, tk), :]
        mg = qk.mfin[tile]
        if (g + lead - DELTA) in qk.ms:
            mg = jnp.where(flag, mg, qk.ms[g + lead - DELTA])
        p = jnp.exp2(s_cur.reshape(tk // 8, 8, tq) - mg[None])
        ls = jnp.sum(p, axis=0)
        l8 = ls if j == 0 else l8 + ls
        pv = jnp.dot(v_ref[:, pl.ds(j * tk, tk)],
                     p.reshape(tk, tq).astype(jnp.bfloat16),
                     preferred_element_type=jnp.float32)
        acc = pv if j == 0 else acc + pv
        if j == nk - 1:
            l = jnp.sum(l8, axis=0, keepdims=True)
            o_ref[:, tile * tq:(tile + 1) * tq] = (acc * (1.0 / l)).astype(o_ref.dtype)
    m_ref[...] = qk.mfin[nq]
    m8_ref[...] = qk.m8


@jax.jit
def pallas_standalone__fused_io_aware_attn__prompt_kernel(
    q: jax.Array,
    k: jax.Array,
    v: jax.Array,
):
    B, H, S, D = q.shape
    BH = B * H
    qT, kT, vT = (jnp.swapaxes(x, -1, -2).reshape(BH, D, S) for x in (q, k, v))
    nxt = lambda t: jnp.minimum(t + 1, BH - 1)
    oT = pl.pallas_call(
        _attn_kernel,
        grid=(BH,),
        in_specs=[
            pl.BlockSpec((None, D, S), lambda t: (t, 0, 0)),
            pl.BlockSpec((None, D, 2 * TQ), lambda t: (nxt(t), 0, 0)),
            pl.BlockSpec((None, D, S), lambda t: (0, 0, 0)),
            pl.BlockSpec((None, D, S), lambda t: (nxt(t), 0, 0)),
            pl.BlockSpec((None, D, S), lambda t: (t, 0, 0)),
        ],
        out_specs=pl.BlockSpec((None, D, S), lambda t: (t, 0, 0)),
        out_shape=jax.ShapeDtypeStruct((BH, D, S), q.dtype),
        scratch_shapes=[
            pltpu.VMEM((2 * S, TQ), jnp.float32),
            pltpu.VMEM((8, TQ), jnp.float32),
            pltpu.VMEM((8, TQ), jnp.float32),
            pltpu.VMEM((S, D), jnp.bfloat16),
            pltpu.VMEM((8, TQ), jnp.int32),
        ],
        compiler_params=pltpu.CompilerParams(
            dimension_semantics=("arbitrary",),
            vmem_limit_bytes=100 * 1024 * 1024),
    )(qT, qT, kT, kT, vT)
    return jnp.swapaxes(oT.reshape(B, H, D, S), -1, -2)
```

```python
import math

import jax
import jax.numpy as jnp
import jax.experimental.pallas as pl
import jax.experimental.pallas.tpu as pltpu

TQ = 512
TK = 128
LAG = 1
FINE = 2


def _attn_kernel(q_ref, qn_ref, k0_ref, kn_ref, v_ref, o_ref,
                 s_ref, m_ref, m8_ref, kt_ref, flag_ref):
    D, S = q_ref.shape
    tq, tk = TQ, TK
    c = (D ** -0.5) * math.log2(math.e)
    t = pl.program_id(0)
    nq = S // tq
    nk = S // tk
    lead = nk + LAG
    ring = 2 * nk
    n_steps = nq * nk
    ng = tk // 16

    class QK:
        def __init__(self, qsrc, ksrc, m8, mfin):
            self.qsrc, self.ksrc, self.m8, self.mfin = qsrc, ksrc, m8, mfin
            self.qcache, self.ms = {}, {}

        def step(self, g):
            tile, j = divmod(g, nk)
            if tile not in self.qcache:
                ref, ti = self.qsrc(tile)
                x = ref[:, ti * tq:(ti + 1) * tq]
                self.qcache[tile] = (x.astype(jnp.float32) * c).astype(jnp.bfloat16)
            ks = self.ksrc(tile)
            sl2 = pl.ds(j * tk // 2, tk // 2)
            if ks is None:
                kc = pltpu.bitcast(kt_ref[sl2, :], jnp.bfloat16)
            else:
                kc = ks[:, pl.ds(j * tk, tk)].T
                kt_ref[sl2, :] = pltpu.bitcast(kc, jnp.uint32)
            s = jnp.dot(kc, self.qcache[tile], preferred_element_type=jnp.float32)
            s_ref[pl.ds((g % ring) * tk, tk), :] = s
            for r in range(ng):
                a = jnp.maximum(s[16 * r:16 * r + 8], s[16 * r + 8:16 * r + 16])
                self.m8 = a if (j == 0 and r == 0) else jnp.maximum(self.m8, a)
                self.ms[g * ng + r] = a
            if j == nk - 1:
                self.mfin[tile] = jnp.broadcast_to(
                    jnp.max(self.m8, axis=0, keepdims=True), (8, tq))

    @pl.when(t == 0)
    def _():
        qk0 = QK(lambda tile: (q_ref, tile),
                 lambda tile: k0_ref if tile == 0 else None, None, {})
        for g in range(lead):
            qk0.step(g)
        m_ref[...] = qk0.mfin[0]
        m8_ref[...] = qk0.m8
        flag_ref[...] = jnp.ones(flag_ref.shape, flag_ref.dtype)

    flag = flag_ref[...] > 0
    qk = QK(lambda tile: (q_ref, tile) if tile < nq else (qn_ref, tile - nq),
            lambda tile: kn_ref if tile == nq else None,
            m8_ref[...], {0: m_ref[...]})
    l8 = acc = None
    for g in range(n_steps):
        tile, j = divmod(g, nk)
        qk.step(g + lead)
        ps = [None] * ng
        for i, r in enumerate(reversed(range(ng))):
            if i % FINE == 0:
                mg = qk.mfin[tile]
                key = (g + lead - 1) * ng + i
                if key in qk.ms:
                    mg = jnp.where(flag, mg, qk.ms[key])
            base = (g % ring) * tk + 16 * r
            pa = jnp.exp2(s_ref[pl.ds(base, 8), :] - mg)
            pb = jnp.exp2(s_ref[pl.ds(base + 8, 8), :] - mg)
            ls = pa + pb
            l8 = ls if (j == 0 and i == 0) else l8 + ls
            ps[r] = jnp.concatenate([pa, pb], axis=0)
        p = jnp.concatenate(ps, axis=0).astype(jnp.bfloat16)
        pv = jnp.dot(v_ref[:, pl.ds(j * tk, tk)], p, preferred_element_type=jnp.float32)
        acc = pv if j == 0 else acc + pv
        if j == nk - 1:
            l = jnp.sum(l8, axis=0, keepdims=True)
            o_ref[:, tile * tq:(tile + 1) * tq] = (acc * (1.0 / l)).astype(o_ref.dtype)
    m_ref[...] = qk.mfin[nq]
    m8_ref[...] = qk.m8


@jax.jit
def pallas_standalone__fused_io_aware_attn__prompt_kernel(
    q: jax.Array,
    k: jax.Array,
    v: jax.Array,
):
    B, H, S, D = q.shape
    BH = B * H
    qT, kT, vT = (jnp.swapaxes(x, -1, -2).reshape(BH, D, S) for x in (q, k, v))
    nxt = lambda t: jnp.minimum(t + 1, BH - 1)
    oT = pl.pallas_call(
        _attn_kernel,
        grid=(BH,),
        in_specs=[
            pl.BlockSpec((None, D, S), lambda t: (t, 0, 0)),
            pl.BlockSpec((None, D, 2 * TQ), lambda t: (nxt(t), 0, 0)),
            pl.BlockSpec((None, D, S), lambda t: (0, 0, 0)),
            pl.BlockSpec((None, D, S), lambda t: (nxt(t), 0, 0)),
            pl.BlockSpec((None, D, S), lambda t: (t, 0, 0)),
        ],
        out_specs=pl.BlockSpec((None, D, S), lambda t: (t, 0, 0)),
        out_shape=jax.ShapeDtypeStruct((BH, D, S), q.dtype),
        scratch_shapes=[
            pltpu.VMEM((2 * S, TQ), jnp.float32),
            pltpu.VMEM((8, TQ), jnp.float32),
            pltpu.VMEM((8, TQ), jnp.float32),
            pltpu.VMEM((S // 2, D), jnp.uint32),
            pltpu.VMEM((8, TQ), jnp.int32),
        ],
        compiler_params=pltpu.CompilerParams(
            dimension_semantics=("arbitrary",),
            vmem_limit_bytes=100 * 1024 * 1024),
    )(qT, qT, kT, kT, vT)
    return jnp.swapaxes(oT.reshape(B, H, D, S), -1, -2)
```

```python
import functools
import math

import jax
import jax.numpy as jnp
from jax import lax
import jax.experimental.pallas as pl
import jax.experimental.pallas.tpu as pltpu

F32, BF16, U32, I32 = jnp.float32, jnp.bfloat16, jnp.uint32, jnp.int32

TQ = 512
TK = 128
KA = 96
EPS = 2.0 ** -11
XMAX = 4
MARGIN = 0.97

Q0, K0, KSTEP, FIN, TIE_LAG, V_TIE, R_TIE, O_TIE = 2, 18, 2, 54, 4, 4, 4, 6


def _attn_kernel(q_hbm, k_hbm, v_hbm, o_hbm,
                 qb_ref, kb_ref, vb_ref, ob_ref, sem,
                 kt_ref, w_ref, vh_ref, p0_ref, l0_ref, up_ref, cw_ref, s_ref):
    BH, D, S = q_hbm.shape
    tq, tk = TQ, TK
    c = (D ** -0.5) * math.log2(math.e)
    nq = S // tq
    nc = S // tk
    ng = tk // 16
    lo0 = D + 16

    def tile4(z):
        return jnp.concatenate([z] * (tq // 128), axis=1)

    def q_copy(h):
        return pltpu.make_async_copy(
            q_hbm.at[jnp.minimum(h, BH - 1)], qb_ref.at[h & 1], sem.at[0, h & 1])

    def k_copy(h):
        return pltpu.make_async_copy(
            k_hbm.at[jnp.minimum(h, BH - 1)], kb_ref.at[h & 3], sem.at[1, h & 1])

    def v_copy(h):
        return pltpu.make_async_copy(
            v_hbm.at[jnp.minimum(h, BH - 1)], vb_ref.at[h & 1], sem.at[2, h & 1])

    def o_copy(h):
        return pltpu.make_async_copy(ob_ref.at[h & 1], o_hbm.at[h], sem.at[3, h & 1])

    def prefetch(h):
        v_copy(h + 1).start()
        q_copy(h + 2).start()
        k_copy(h + 2).start()

    def pack_lhs(ks):
        row = lax.broadcasted_iota(I32, (8, tk), 0)
        lane = lax.broadcasted_iota(I32, (8, KA), 1)
        e0 = jnp.where(row == 0, 1.0, 0.0)
        e01 = jnp.where(row < 2, 1.0, 0.0)
        aug = jnp.concatenate(
            [ks, e0, e0, ks * EPS, e01, jnp.zeros_like(e0)], axis=0).astype(BF16)
        z = pltpu.bitcast(aug.T, U32)
        out = []
        for i in range(ng // 2):
            hi_g, lo_g = ng - 1 - 2 * i, ng - 2 - 2 * i
            out.append(jnp.where(lane < lo0, z[8 * hi_g:8 * hi_g + 8],
                                 z[8 * lo_g:8 * lo_g + 8]))
        return out

    def prep_k(hn, ci, run):
        ks = kb_ref[hn & 3, :, pl.ds(ci * tk, tk)].astype(F32) * c
        for i, zz in enumerate(pack_lhs(ks)):
            kt_ref[hn & 1, pl.ds(ci * 32 + 8 * i, 8), :] = zz
        n2 = jnp.sum(ks * ks, axis=0, keepdims=True)
        return n2 if run is None else jnp.maximum(run, n2)

    def prep_q(hn, i, run):
        qb = qb_ref[hn & 1, :, i * 128:(i + 1) * 128]
        ti, off = divmod(i * 128, tq)
        w_ref[hn & 1, ti, :, off:off + 128] = pltpu.bitcast(qb, U32)
        x = qb.astype(F32)
        n2 = jnp.sum(x * x, axis=0, keepdims=True)
        return n2 if run is None else jnp.maximum(run, n2)

    def scale_from(rq, rk):
        mq = jnp.max(rq, axis=1, keepdims=True) + 2.0 ** -100
        mk = jnp.max(rk, axis=1, keepdims=True) + 2.0 ** -100
        b2 = jnp.broadcast_to(mq * mk, (8, 128))
        p2 = jnp.full((8, 128), 2.0 ** XMAX, F32)
        up = jnp.full((8, 128), 2.0 ** (2 ** XMAX), F32)
        for x in reversed(range(XMAX)):
            ok = b2 <= (MARGIN * 2.0 ** (x - 1)) ** 2
            p2 = jnp.where(ok, 2.0 ** x, p2)
            up = jnp.where(ok, 2.0 ** (2 ** x), up)
        fast = jnp.where(b2 <= (MARGIN * 2.0 ** (XMAX - 1)) ** 2, 1, 0).astype(I32)
        return p2, up, fast

    def const_rows(p2):
        row = lax.broadcasted_iota(I32, (8, 128), 0)
        a0 = jnp.where(row == 0, 1.5 * 2.0 ** 12, 0.0) * p2
        b0 = jnp.where(row == 0, -1.5, jnp.where(row == 1, -(2.0 ** -12), 0.0)) * p2
        wa = jnp.concatenate([a0, -a0], axis=0).astype(BF16)
        wb = jnp.concatenate([b0, jnp.zeros_like(b0)], axis=0).astype(BF16)
        return pltpu.bitcast(wa, U32), pltpu.bitcast(wb, U32)

    def packed_dot(kc, wq, consts):
        w = jnp.concatenate([wq, tile4(consts[0]), wq, tile4(consts[1])], axis=0)
        return jnp.dot(pltpu.bitcast(kc, BF16), pltpu.bitcast(w, BF16),
                       preferred_element_type=F32)

    def qk(b, tile, ci, consts):
        return packed_dot(kt_ref[b, pl.ds(ci * 32, 32), :], w_ref[b, tile], consts)

    def decode(tt):
        hi = pltpu.bitcast(pltpu.bitcast(tt, U32) & jnp.uint32(0xFFFFF000), F32)
        return hi, (tt - hi) * (1.0 / EPS)

    def exp_chunk(tt, lh, ll):
        grp = [None] * ng
        for i in range(ng // 2):
            ph, plo = [], []
            for u in range(2):
                r0 = 16 * i + 8 * u
                hi, lo = decode(tt[r0:r0 + 8])
                ph.append(jnp.exp2(hi))
                plo.append(jnp.exp2(lo))
            a = ph[0] + ph[1]
            b = plo[0] + plo[1]
            lh = a if lh is None else lh + a
            ll = b if ll is None else ll + b
            grp[ng - 1 - 2 * i] = jnp.concatenate(ph, axis=0)
            grp[ng - 2 - 2 * i] = jnp.concatenate(plo, axis=0)
        return jnp.concatenate(grp, axis=0).astype(BF16), lh, ll

    def finish_prep(tt0, nconsts, up):
        lh = ll = None
        for e in range(2):
            p, lh, ll = exp_chunk(tt0[e], lh, ll)
            p0_ref[e] = p
        l0_ref[0] = lh
        l0_ref[1] = ll
        up_ref[...] = up
        cw_ref[0] = nconsts[0]
        cw_ref[1] = nconsts[1]

    def full_prep(hn):
        rq = rk = None
        for i in range(nc):
            rq = prep_q(hn, i, rq)
        for ci in range(nc):
            rk = prep_k(hn, ci, rk)
        p2, up, nfast = scale_from(rq, rk)
        nconsts = const_rows(p2)
        finish_prep([qk(hn & 1, 0, e, nconsts) for e in range(2)], nconsts, up)
        return nfast[0, 0]

    def probe():
        r = lax.broadcasted_iota(I32, (D, tk), 0)
        cc = lax.broadcasted_iota(I32, (D, tk), 1)
        ks = (((r * 37 + cc * 11) & 127) - 63).astype(F32) * (2.0 ** -9)
        r = lax.broadcasted_iota(I32, (D, tq), 0)
        cc = lax.broadcasted_iota(I32, (D, tq), 1)
        qs = ((((r * 29 + cc * 13) & 127) - 63).astype(F32) * (2.0 ** -10)).astype(BF16)
        kc = jnp.concatenate(pack_lhs(ks), axis=0)
        tt = packed_dot(kc, pltpu.bitcast(qs, U32), const_rows(jnp.ones((8, 128), F32)))
        hi, lo = decode(tt)
        ex = lax.dot_general(ks.astype(BF16), qs, (((0,), (0,)), ((), ())),
                             preferred_element_type=F32)
        err = None
        for i in range(ng // 2):
            hi_g, lo_g = ng - 1 - 2 * i, ng - 2 - 2 * i
            e1 = jnp.abs(hi[16 * i:16 * i + 16] + 1.5 - ex[16 * hi_g:16 * hi_g + 16])
            e2 = jnp.abs(lo[16 * i:16 * i + 16] + 0.5 - ex[16 * lo_g:16 * lo_g + 16])
            e = jnp.maximum(e1, e2)
            err = e if err is None else jnp.maximum(err, e)
        bad = jnp.where(err <= 2.0 ** -11, 0.0, 1.0)
        return jnp.where(jnp.max(bad) == 0.0, 1, 0).astype(I32)

    def slow_head(h):
        prefetch(h)
        cur = h & 1

        def tile_body(tile, carry):
            wq = pltpu.bitcast(w_ref[cur, tile], BF16)
            m8 = None
            for ci in range(nc):
                s = lax.dot_general(kb_ref[h & 3, :, pl.ds(ci * tk, tk)], wq,
                                    (((0,), (0,)), ((), ())),
                                    preferred_element_type=F32) * c
                s_ref[pl.ds(ci * tk, tk), :] = s
                mm = jnp.max(s.reshape(tk // 8, 8, tq), axis=0)
                m8 = mm if m8 is None else jnp.maximum(m8, mm)
            m = jnp.broadcast_to(jnp.max(m8, axis=0, keepdims=True), (8, tq))
            l8 = acc = None
            for ci in range(nc):
                ps = [None] * ng
                for r in reversed(range(ng)):
                    pa = jnp.exp2(s_ref[pl.ds(ci * tk + 16 * r, 8), :] - m)
                    pb = jnp.exp2(s_ref[pl.ds(ci * tk + 16 * r + 8, 8), :] - m)
                    l8 = pa + pb if l8 is None else l8 + (pa + pb)
                    ps[r] = jnp.concatenate([pa, pb], axis=0)
                p = jnp.concatenate(ps, axis=0).astype(BF16)
                pv = jnp.dot(vb_ref[cur, :, pl.ds(ci * tk, tk)], p,
                             preferred_element_type=F32)
                acc = pv if acc is None else acc + pv
            l = jnp.sum(l8, axis=0, keepdims=True)
            off = pl.multiple_of(tile * tq, tq)
            ob_ref[cur, :, pl.ds(off, tq)] = (acc * (1.0 / l)).astype(ob_ref.dtype)
            return carry

        lax.fori_loop(0, nq, tile_body, 0)
        return full_prep(h + 1)

    def fast_head(h):
        prefetch(h)
        cur = h & 1
        hn = h + 1
        consts = (cw_ref[0], cw_ref[1])
        up = up_ref[...]
        lane = lax.broadcasted_iota(I32, (8, tk), 1)
        upv = jnp.where((lane // 16) % 2 == 1, up, 1.0)

        always = up > 0.0
        ties = {}

        def tie(e, val):
            if val.dtype != U32:
                val = pltpu.bitcast(jnp.broadcast_to(val, (8, 128)), U32)
            ties.setdefault(e, []).append(val)

        for ci in range(nc):
            vf = vb_ref[cur, :, pl.ds(ci * tk, tk)].astype(F32)
            vf = (vf.reshape(D // 8, 8, tk) * upv[None]).reshape(D, tk)
            vhu = pltpu.bitcast(vf.astype(BF16), U32)
            vh_ref[:, pl.ds(ci * tk, tk)] = vhu
            if V_TIE < ci + 2:
                tie(V_TIE, vhu[0:8])
                tie(V_TIE, vhu[8:16])

        n_steps = nq * nc
        tts, tt0 = {}, []
        lh = ll = acc = rq = rk = nxt = nconsts = None
        for e in range(n_steps):
            tile, ci = divmod(e, nc)
            if e + 2 < n_steps:
                t1, c1 = divmod(e + 2, nc)
                cb = consts[1]
                vals = ties.pop(e + 2, [])
                if vals:
                    cb = jnp.where(always, cb, functools.reduce(jnp.bitwise_or, vals))
                tts[e + 2] = qk(cur, t1, c1, (consts[0], cb))
            else:
                tt0.append(qk(hn & 1, 0, e + 2 - n_steps, nconsts))
            if 0 <= e - Q0 < nc:
                rq = prep_q(hn, e - Q0, rq)
                tie(e + TIE_LAG, rq)
            if (e - K0) % KSTEP == 0 and 0 <= (e - K0) // KSTEP < nc:
                rk = prep_k(hn, (e - K0) // KSTEP, rk)
                tie(e + TIE_LAG, rk)
            if e == FIN:
                nxt = scale_from(rq, rk)
                nconsts = const_rows(nxt[0])
                tie(e + TIE_LAG, nconsts[0])
                tie(e + TIE_LAG, nconsts[1])
            if ci == 0:
                lh = ll = None
            if e == 0:
                lh, ll = l0_ref[0], l0_ref[1]
            if e < 2:
                p = p0_ref[e]
            else:
                p, lh, ll = exp_chunk(tts.pop(e), lh, ll)
            vh = pltpu.bitcast(vh_ref[:, pl.ds(ci * tk, tk)], BF16)
            pv = jnp.dot(vh, p, preferred_element_type=F32)
            acc = pv if ci == 0 else acc + pv
            if ci == nc - 1:
                l = jnp.sum(lh * tile4(up) + ll, axis=0, keepdims=True)
                rinv = 1.0 / l
                of = acc * rinv
                for u in range(tq // 128):
                    tie(e + R_TIE, rinv[:, u * 128:(u + 1) * 128])
                    tie(e + O_TIE, of[D - 8:D, u * 128:(u + 1) * 128])
                ob_ref[cur, :, tile * tq:(tile + 1) * tq] = of.astype(ob_ref.dtype)
        finish_prep(tt0, nconsts, nxt[1])
        return nxt[2][0, 0]

    zero = jnp.int32(0)
    q_copy(zero).start()
    k_copy(zero).start()
    v_copy(zero).start()
    q_copy(zero + 1).start()
    k_copy(zero + 1).start()
    ok = probe()
    q_copy(zero).wait()
    k_copy(zero).wait()
    fast0 = full_prep(zero) * ok

    def body(h, fast):
        v_copy(h).wait()
        q_copy(h + 1).wait()
        k_copy(h + 1).wait()

        @pl.when(h >= 2)
        def _():
            o_copy(h - 2).wait()

        nfast = lax.cond(fast == 1, fast_head, slow_head, h)
        o_copy(h).start()
        return nfast * ok

    lax.fori_loop(0, BH, body, fast0)
    last = jnp.int32(BH)
    v_copy(last).wait()
    q_copy(last + 1).wait()
    k_copy(last + 1).wait()
    o_copy(last - 2).wait()
    o_copy(last - 1).wait()


@jax.jit
def pallas_standalone__fused_io_aware_attn__prompt_kernel(
    q: jax.Array,
    k: jax.Array,
    v: jax.Array,
):
    B, H, S, D = q.shape
    BH = B * H
    qT, kT, vT = (jnp.swapaxes(x, -1, -2).reshape(BH, D, S) for x in (q, k, v))
    hbm = pl.BlockSpec(memory_space=pl.ANY)
    oT = pl.pallas_call(
        _attn_kernel,
        in_specs=[hbm, hbm, hbm],
        out_specs=hbm,
        out_shape=jax.ShapeDtypeStruct((BH, D, S), q.dtype),
        scratch_shapes=[
            pltpu.VMEM((2, D, S), BF16),
            pltpu.VMEM((4, D, S), BF16),
            pltpu.VMEM((2, D, S), BF16),
            pltpu.VMEM((2, D, S), BF16),
            pltpu.SemaphoreType.DMA((4, 2)),
            pltpu.VMEM((2, S // 4, KA), U32),
            pltpu.VMEM((2, S // TQ, D // 2, TQ), U32),
            pltpu.VMEM((D // 2, S), U32),
            pltpu.VMEM((2, TK, TQ), BF16),
            pltpu.VMEM((2, 8, TQ), F32),
            pltpu.VMEM((8, 128), F32),
            pltpu.VMEM((2, 8, 128), U32),
            pltpu.VMEM((S, TQ), F32),
        ],
        compiler_params=pltpu.CompilerParams(
            disable_bounds_checks=True,
            vmem_limit_bytes=64 * 1024 * 1024),
    )(qT, kT, vT)
    return jnp.swapaxes(oT.reshape(B, H, D, S), -1, -2)
```

```python
import functools
import math

import jax
import jax.numpy as jnp
from jax import lax
import jax.experimental.pallas as pl
import jax.experimental.pallas.tpu as pltpu

F32, BF16, U32, I32 = jnp.float32, jnp.bfloat16, jnp.uint32, jnp.int32

HB = 2
TQ = 512
TK = 128
KA = 96
EPS = 2.0 ** -11
XMAX = 4
MARGIN = 0.97

Q0, K0, KSTEP, V0, VSTEP, FIN = 19, 10, 3, 5, 3, 56
TIE_LAG, V_TIE, V_PROG, R_TIE, O_TIE = 4, 3, 2, 4, 6


def _attn_kernel(q_hbm, k_hbm, v_hbm, o_hbm,
                 qb_ref, kb_ref, vb_ref, ob_ref, sem,
                 kt_ref, w_ref, vh_ref, p0_ref, l0_ref, up_ref, cw_ref,
                 s_ref, kr_ref):
    NB, _, D, S = q_hbm.shape
    tq, tk = TQ, TK
    c = (D ** -0.5) * math.log2(math.e)
    nq = S // tq
    nc = S // tk
    ng = tk // 16
    lo0 = D + 16

    def tile4(z):
        return jnp.concatenate([z] * (tq // 128), axis=1)

    def q_copy(b):
        return pltpu.make_async_copy(
            q_hbm.at[jnp.minimum(b, NB - 1)], qb_ref.at[b & 1], sem.at[0, b & 1])

    def k_copy(b):
        return pltpu.make_async_copy(
            k_hbm.at[jnp.minimum(b, NB - 1)], kb_ref.at[b & 3], sem.at[1, b & 1])

    def v_copy(b):
        return pltpu.make_async_copy(
            v_hbm.at[jnp.minimum(b, NB - 1)], vb_ref.at[b & 1], sem.at[2, b & 1])

    def o_copy(b):
        return pltpu.make_async_copy(ob_ref.at[b & 1], o_hbm.at[b], sem.at[3, b & 1])

    def prefetch(b):
        v_copy(b + 1).start()
        q_copy(b + 2).start()
        k_copy(b + 2).start()

    def pack_lhs(ks):
        row = lax.broadcasted_iota(I32, (8, tk), 0)
        lane = lax.broadcasted_iota(I32, (8, KA), 1)
        e0 = jnp.where(row == 0, 1.0, 0.0)
        e01 = jnp.where(row < 2, 1.0, 0.0)
        aug = jnp.concatenate(
            [ks, e0, e0, ks * EPS, e01, jnp.zeros_like(e0)], axis=0).astype(BF16)
        z = pltpu.bitcast(aug.T, U32)
        out = []
        for i in range(ng // 2):
            hi_g, lo_g = ng - 1 - 2 * i, ng - 2 - 2 * i
            out.append(jnp.where(lane < lo0, z[8 * hi_g:8 * hi_g + 8],
                                 z[8 * lo_g:8 * lo_g + 8]))
        return out

    def prep_k(bn, j, ci, run):
        ks = kb_ref[bn & 3, j, :, pl.ds(ci * tk, tk)].astype(F32) * c
        for i, zz in enumerate(pack_lhs(ks)):
            kt_ref[bn & 1, j, pl.ds(ci * 32 + 8 * i, 8), :] = zz
        n2 = jnp.sum(ks * ks, axis=0, keepdims=True)
        return n2 if run is None else jnp.maximum(run, n2)

    def prep_q(bn, j, i, run):
        qb = qb_ref[bn & 1, j, :, i * 128:(i + 1) * 128]
        ti, off = divmod(i * 128, tq)
        w_ref[bn & 1, j, ti, :, off:off + 128] = pltpu.bitcast(qb, U32)
        x = qb.astype(F32)
        n2 = jnp.sum(x * x, axis=0, keepdims=True)
        return n2 if run is None else jnp.maximum(run, n2)

    def const_rows(p2):
        row = lax.broadcasted_iota(I32, (8, 128), 0)
        a0 = jnp.where(row == 0, 1.5 * 2.0 ** 12, 0.0) * p2
        b0 = jnp.where(row == 0, -1.5, jnp.where(row == 1, -(2.0 ** -12), 0.0)) * p2
        wa = jnp.concatenate([a0, -a0], axis=0).astype(BF16)
        wb = jnp.concatenate([b0, jnp.zeros_like(b0)], axis=0).astype(BF16)
        return pltpu.bitcast(wa, U32), pltpu.bitcast(wb, U32)

    def prep_scale(bn, j, rq, rk):
        mq = jnp.max(rq, axis=1, keepdims=True) + 2.0 ** -100
        mk = jnp.max(rk, axis=1, keepdims=True) + 2.0 ** -100
        b2 = jnp.broadcast_to(mq * mk, (8, 128))
        p2 = jnp.full((8, 128), 2.0 ** XMAX, F32)
        up = jnp.full((8, 128), 2.0 ** (2 ** XMAX), F32)
        for x in reversed(range(XMAX)):
            ok = b2 <= (MARGIN * 2.0 ** (x - 1)) ** 2
            p2 = jnp.where(ok, 2.0 ** x, p2)
            up = jnp.where(ok, 2.0 ** (2 ** x), up)
        fast = jnp.where(b2 <= (MARGIN * 2.0 ** (XMAX - 1)) ** 2, 1, 0).astype(I32)
        consts = const_rows(p2)
        up_ref[bn & 1, j] = up
        cw_ref[bn & 1, j, 0] = consts[0]
        cw_ref[bn & 1, j, 1] = consts[1]
        return consts, fast

    def packed_dot(kc, wq, consts):
        w = jnp.concatenate([wq, tile4(consts[0]), wq, tile4(consts[1])], axis=0)
        return jnp.dot(pltpu.bitcast(kc, BF16), pltpu.bitcast(w, BF16),
                       preferred_element_type=F32)

    def qk(slot, j, tile, ci, consts):
        return packed_dot(kt_ref[slot, j, pl.ds(ci * 32, 32), :],
                          w_ref[slot, j, tile], consts)

    def decode(tt):
        hi = pltpu.bitcast(pltpu.bitcast(tt, U32) & jnp.uint32(0xFFFFF000), F32)
        return hi, (tt - hi) * (1.0 / EPS)

    def exp_chunk(tt, lh, ll):
        grp = [None] * ng
        for i in range(ng // 2):
            ph, plo = [], []
            for u in range(2):
                r0 = 16 * i + 8 * u
                hi, lo = decode(tt[r0:r0 + 8])
                ph.append(jnp.exp2(hi))
                plo.append(jnp.exp2(lo))
            a = ph[0] + ph[1]
            b = plo[0] + plo[1]
            lh = a if lh is None else lh + a
            ll = b if ll is None else ll + b
            grp[ng - 1 - 2 * i] = jnp.concatenate(ph, axis=0)
            grp[ng - 2 - 2 * i] = jnp.concatenate(plo, axis=0)
        return jnp.concatenate(grp, axis=0).astype(BF16), lh, ll

    def store_carry(tt0):
        lh = ll = None
        for e in range(2):
            p, lh, ll = exp_chunk(tt0[e], lh, ll)
            p0_ref[e] = p
        l0_ref[0] = lh
        l0_ref[1] = ll

    def full_prep(bn):
        allfast = None
        for j in range(HB):
            rq = rk = None
            for i in range(nc):
                rq = prep_q(bn, j, i, rq)
            for ci in range(nc):
                rk = prep_k(bn, j, ci, rk)
            consts, fast = prep_scale(bn, j, rq, rk)
            if j == 0:
                store_carry([qk(bn & 1, 0, 0, e, consts) for e in range(2)])
            allfast = fast if allfast is None else allfast * fast
        return allfast[0, 0]

    def probe():
        r = lax.broadcasted_iota(I32, (D, tk), 0)
        cc = lax.broadcasted_iota(I32, (D, tk), 1)
        ks = (((r * 37 + cc * 11) & 127) - 63).astype(F32) * (2.0 ** -9)
        r = lax.broadcasted_iota(I32, (D, tq), 0)
        cc = lax.broadcasted_iota(I32, (D, tq), 1)
        qs = ((((r * 29 + cc * 13) & 127) - 63).astype(F32) * (2.0 ** -10)).astype(BF16)
        kc = jnp.concatenate(pack_lhs(ks), axis=0)
        tt = packed_dot(kc, pltpu.bitcast(qs, U32), const_rows(jnp.ones((8, 128), F32)))
        hi, lo = decode(tt)
        ex = lax.dot_general(ks.astype(BF16), qs, (((0,), (0,)), ((), ())),
                             preferred_element_type=F32)
        err = None
        for i in range(ng // 2):
            hi_g, lo_g = ng - 1 - 2 * i, ng - 2 - 2 * i
            e1 = jnp.abs(hi[16 * i:16 * i + 16] + 1.5 - ex[16 * hi_g:16 * hi_g + 16])
            e2 = jnp.abs(lo[16 * i:16 * i + 16] + 0.5 - ex[16 * lo_g:16 * lo_g + 16])
            e = jnp.maximum(e1, e2)
            err = e if err is None else jnp.maximum(err, e)
        bad = jnp.where(err <= 2.0 ** -11, 0.0, 1.0)
        return jnp.where(jnp.max(bad) == 0.0, 1, 0).astype(I32)

    def exact_block(b):
        prefetch(b)
        cur = b & 1
        n_tiles = HB * nq
        always = tile4(up_ref[cur, 0]) > 0.0
        for j in range(HB):
            for ci in range(nc):
                kr_ref[j, pl.ds(ci * 64, 64), :] = pltpu.bitcast(
                    kb_ref[b & 3, j, :, pl.ds(ci * tk, tk)].T, U32)

        def stage(it_qk, it_pv, m):
            if it_qk is not None:
                jq = it_qk // nq
                wq = pltpu.bitcast(w_ref[cur, jq, it_qk % nq], BF16)
            if it_pv is not None:
                jv = it_pv // nq
            m8 = l8 = acc = prev = None
            for ci in range(nc):
                if it_pv is not None:
                    s_cur = s_ref[pl.ds(ci * tk, tk), :]
                cm = None
                if it_qk is not None:
                    kc = pltpu.bitcast(kr_ref[jq, pl.ds(ci * 64, 64), :], BF16)
                    s = jnp.dot(kc, wq, preferred_element_type=F32)
                    s_ref[pl.ds(ci * tk, tk), :] = s
                    cm = [jnp.maximum(s[16 * r:16 * r + 8], s[16 * r + 8:16 * r + 16])
                          for r in range(ng)]
                    for a in cm:
                        m8 = a if m8 is None else jnp.maximum(m8, a)
                if it_pv is not None:
                    ps = [None] * ng
                    for i, r in enumerate(reversed(range(ng))):
                        if i % 2 == 0:
                            mg = m if prev is None else jnp.where(always, m, prev[i])
                        pa = jnp.exp2((s_cur[16 * r:16 * r + 8] - mg) * c)
                        pb = jnp.exp2((s_cur[16 * r + 8:16 * r + 16] - mg) * c)
                        l8 = pa + pb if l8 is None else l8 + (pa + pb)
                        ps[r] = jnp.concatenate([pa, pb], axis=0)
                    p = jnp.concatenate(ps, axis=0).astype(BF16)
                    pv = jnp.dot(vb_ref[cur, jv, :, pl.ds(ci * tk, tk)], p,
                                 preferred_element_type=F32)
                    acc = pv if acc is None else acc + pv
                prev = cm
            if it_pv is not None:
                l = jnp.sum(l8, axis=0, keepdims=True)
                off = pl.multiple_of((it_pv % nq) * tq, tq)
                ob_ref[cur, jv, :, pl.ds(off, tq)] = (acc * (1.0 / l)).astype(ob_ref.dtype)
            if it_qk is None:
                return None
            return jnp.broadcast_to(jnp.max(m8, axis=0, keepdims=True), (8, tq))

        m = stage(0, None, None)
        m = lax.fori_loop(0, n_tiles - 1, lambda i, mm: stage(i + 1, i, mm), m)
        stage(None, n_tiles - 1, m)
        return full_prep(b + 1)

    def packed_block(b):
        cur = b & 1
        bn = b + 1
        consts = [(cw_ref[cur, j, 0], cw_ref[cur, j, 1]) for j in range(HB)]
        ups = [up_ref[cur, j] for j in range(HB)]
        lane = lax.broadcasted_iota(I32, (8, tk), 1)
        odd = (lane // 16) % 2 == 1

        always = ups[0] > 0.0
        ties = {}

        def tie(e, val):
            if val.dtype != U32:
                val = pltpu.bitcast(jnp.broadcast_to(val, (8, 128)), U32)
            ties.setdefault(e, []).append(val)

        def prep_v(j, ci, e_tie):
            upv = jnp.where(odd, ups[j], 1.0)
            vf = vb_ref[cur, j, :, pl.ds(ci * tk, tk)].astype(F32)
            vf = (vf.reshape(D // 8, 8, tk) * upv[None]).reshape(D, tk)
            vhu = pltpu.bitcast(vf.astype(BF16), U32)
            vh_ref[j, :, pl.ds(ci * tk, tk)] = vhu
            if e_tie is not None:
                tie(e_tie, vhu[0:8])
                tie(e_tie, vhu[8:16])

        per_head = nq * nc
        n_steps = HB * per_head
        tts, tt0, runs = {}, [], []
        lh = ll = acc = rq = rk = allfast = nconsts0 = None
        for e in range(n_steps):
            j, el = divmod(e, per_head)
            tile, ci = divmod(el, nc)
            if e + 2 < n_steps:
                j1, el1 = divmod(e + 2, per_head)
                t1, c1 = divmod(el1, nc)
                cb = consts[j1][1]
                vals = ties.pop(e + 2, [])
                if vals:
                    cb = jnp.where(always, cb, functools.reduce(jnp.bitwise_or, vals))
                tts[e + 2] = qk(cur, j1, t1, c1, (consts[j1][0], cb))
            else:
                tt0.append(qk(bn & 1, 0, 0, e + 2 - n_steps, nconsts0))
            if e == 0:
                prefetch(b)
                for cv in range(nc):
                    et = V_TIE + cv // V_PROG
                    prep_v(0, cv, et if et < cv + 2 else None)
            jp = (j + 1) % HB
            if el == 0:
                rq = rk = None
            if 0 <= el - Q0 < nc:
                rq = prep_q(bn, jp, el - Q0, rq)
                tie(e + TIE_LAG, rq)
            if (el - K0) % KSTEP == 0 and 0 <= (el - K0) // KSTEP < nc:
                rk = prep_k(bn, jp, (el - K0) // KSTEP, rk)
                tie(e + TIE_LAG, rk)
            if j + 1 < HB and (el - V0) % VSTEP == 0 and 0 <= (el - V0) // VSTEP < nc:
                prep_v(j + 1, (el - V0) // VSTEP, e + TIE_LAG)
            if el == FIN:
                runs.append((jp, rq, rk))
                if j == HB - 1:
                    for jn, rqn, rkn in runs:
                        nconsts, fast = prep_scale(bn, jn, rqn, rkn)
                        tie(e + TIE_LAG, nconsts[0])
                        tie(e + TIE_LAG, nconsts[1])
                        if jn == 0:
                            nconsts0 = nconsts
                        allfast = fast if allfast is None else allfast * fast
            if ci == 0:
                lh = ll = None
            if e == 0:
                lh, ll = l0_ref[0], l0_ref[1]
            if e < 2:
                p = p0_ref[e]
            else:
                p, lh, ll = exp_chunk(tts.pop(e), lh, ll)
            vh = pltpu.bitcast(vh_ref[j, :, pl.ds(ci * tk, tk)], BF16)
            pv = jnp.dot(vh, p, preferred_element_type=F32)
            acc = pv if ci == 0 else acc + pv
            if ci == nc - 1:
                l = jnp.sum(lh * tile4(ups[j]) + ll, axis=0, keepdims=True)
                r0 = pl.reciprocal(l, approx=True)
                rinv = r0 * (2.0 - l * r0)
                of = acc * rinv
                for u in range(tq // 128):
                    tie(e + R_TIE, rinv[:, u * 128:(u + 1) * 128])
                    tie(e + O_TIE, of[D - 8:D, u * 128:(u + 1) * 128])
                ob_ref[cur, j, :, tile * tq:(tile + 1) * tq] = of.astype(ob_ref.dtype)
        store_carry(tt0)
        return allfast[0, 0]

    zero = jnp.int32(0)
    q_copy(zero).start()
    k_copy(zero).start()
    v_copy(zero).start()
    q_copy(zero + 1).start()
    k_copy(zero + 1).start()
    ok = probe()
    q_copy(zero).wait()
    k_copy(zero).wait()
    fast0 = full_prep(zero) * ok

    def body(b, fast):
        @pl.when(b >= 1)
        def _():
            o_copy(b - 1).start()

        v_copy(b).wait()
        q_copy(b + 1).wait()
        k_copy(b + 1).wait()

        @pl.when(b >= 2)
        def _():
            o_copy(b - 2).wait()

        return lax.cond(fast == 1, packed_block, exact_block, b) * ok

    lax.fori_loop(0, NB, body, fast0)
    last = jnp.int32(NB)
    o_copy(last - 1).start()
    v_copy(last).wait()
    q_copy(last + 1).wait()
    k_copy(last + 1).wait()
    o_copy(last - 2).wait()
    o_copy(last - 1).wait()


@jax.jit
def pallas_standalone__fused_io_aware_attn__prompt_kernel(
    q: jax.Array,
    k: jax.Array,
    v: jax.Array,
):
    B, H, S, D = q.shape
    NB = B * H // HB
    qT, kT, vT = (jnp.swapaxes(x, -1, -2).reshape(NB, HB, D, S) for x in (q, k, v))
    hbm = pl.BlockSpec(memory_space=pl.ANY)
    oT = pl.pallas_call(
        _attn_kernel,
        in_specs=[hbm, hbm, hbm],
        out_specs=hbm,
        out_shape=jax.ShapeDtypeStruct((NB, HB, D, S), q.dtype),
        scratch_shapes=[
            pltpu.VMEM((2, HB, D, S), BF16),
            pltpu.VMEM((4, HB, D, S), BF16),
            pltpu.VMEM((2, HB, D, S), BF16),
            pltpu.VMEM((2, HB, D, S), BF16),
            pltpu.SemaphoreType.DMA((4, 2)),
            pltpu.VMEM((2, HB, S // 4, KA), U32),
            pltpu.VMEM((2, HB, S // TQ, D // 2, TQ), U32),
            pltpu.VMEM((HB, D // 2, S), U32),
            pltpu.VMEM((2, TK, TQ), BF16),
            pltpu.VMEM((2, 8, TQ), F32),
            pltpu.VMEM((2, HB, 8, 128), F32),
            pltpu.VMEM((2, HB, 2, 8, 128), U32),
            pltpu.VMEM((S, TQ), F32),
            pltpu.VMEM((HB, S // 2, D), U32),
        ],
        compiler_params=pltpu.CompilerParams(
            disable_bounds_checks=True,
            vmem_limit_bytes=64 * 1024 * 1024),
    )(qT, kT, vT)
    return jnp.swapaxes(oT.reshape(B, H, D, S), -1, -2)
```

```python
import functools
import math

import jax
import jax.numpy as jnp
from jax import lax
import jax.experimental.pallas as pl
import jax.experimental.pallas.tpu as pltpu

F32, BF16, U32, I32 = jnp.float32, jnp.bfloat16, jnp.uint32, jnp.int32

HB = 2
TQ = 512
TK = 128
KA = 96
EPS = 2.0 ** -11
XMAX = 4
MARGIN = 0.97

Q0, QSTEP, K0, KSTEP, V0, VSTEP, FIN = 19, 1, 10, 3, 8, 3, 57
TIE_LAG, V_TIE, V_PROG, R_TIE, O_TIE = 4, 3, 2, 4, 6


def _attn_kernel(q_hbm, k_hbm, v_hbm, o_hbm,
                 qb_ref, kb_ref, vb_ref, ob_ref, sem,
                 kt_ref, w_ref, vh_ref, p0_ref, l0_ref, up_ref, cw_ref,
                 s_ref, kr_ref):
    NB, _, D, S = q_hbm.shape
    tq, tk = TQ, TK
    c = (D ** -0.5) * math.log2(math.e)
    nq = S // tq
    nc = S // tk
    ng = tk // 16
    lo0 = D + 16

    def tile4(z):
        return jnp.concatenate([z] * (tq // 128), axis=1)

    def q_copy(b):
        return pltpu.make_async_copy(
            q_hbm.at[jnp.minimum(b, NB - 1)], qb_ref.at[b & 1], sem.at[0, b & 1])

    def k_copy(b):
        return pltpu.make_async_copy(
            k_hbm.at[jnp.minimum(b, NB - 1)], kb_ref.at[b & 3], sem.at[1, b & 1])

    def v_copy(b):
        return pltpu.make_async_copy(
            v_hbm.at[jnp.minimum(b, NB - 1)], vb_ref.at[b & 1], sem.at[2, b & 1])

    def o_copy(b, j):
        return pltpu.make_async_copy(
            ob_ref.at[b & 1, j], o_hbm.at[b, j], sem.at[3 + j, b & 1])

    def prefetch(b):
        v_copy(b + 1).start()
        q_copy(b + 2).start()
        k_copy(b + 2).start()

    def pack_lhs(ks):
        row = lax.broadcasted_iota(I32, (8, tk), 0)
        lane = lax.broadcasted_iota(I32, (8, KA), 1)
        e0 = jnp.where(row == 0, 1.0, 0.0)
        e01 = jnp.where(row < 2, 1.0, 0.0)
        aug = jnp.concatenate(
            [ks, e0, e0, ks * EPS, e01, jnp.zeros_like(e0)], axis=0).astype(BF16)
        z = pltpu.bitcast(aug.T, U32)
        out = []
        for i in range(ng // 2):
            hi_g, lo_g = ng - 1 - 2 * i, ng - 2 - 2 * i
            out.append(jnp.where(lane < lo0, z[8 * hi_g:8 * hi_g + 8],
                                 z[8 * lo_g:8 * lo_g + 8]))
        return out

    def prep_k(bn, j, ci, run):
        ks = kb_ref[bn & 3, j, :, pl.ds(ci * tk, tk)].astype(F32) * c
        for i, zz in enumerate(pack_lhs(ks)):
            kt_ref[bn & 1, j, pl.ds(ci * 32 + 8 * i, 8), :] = zz
        n2 = jnp.sum(ks * ks, axis=0, keepdims=True)
        return n2 if run is None else jnp.maximum(run, n2)

    def prep_q(bn, j, i, run):
        qb = qb_ref[bn & 1, j, :, i * 128:(i + 1) * 128]
        ti, off = divmod(i * 128, tq)
        w_ref[bn & 1, j, ti, :, off:off + 128] = pltpu.bitcast(qb, U32)
        x = qb.astype(F32)
        n2 = jnp.sum(x * x, axis=0, keepdims=True)
        return n2 if run is None else jnp.maximum(run, n2)

    def const_rows(p2):
        row = lax.broadcasted_iota(I32, (8, 128), 0)
        a0 = jnp.where(row == 0, 1.5 * 2.0 ** 12, 0.0) * p2
        b0 = jnp.where(row == 0, -1.5, jnp.where(row == 1, -(2.0 ** -12), 0.0)) * p2
        wa = jnp.concatenate([a0, -a0], axis=0).astype(BF16)
        wb = jnp.concatenate([b0, jnp.zeros_like(b0)], axis=0).astype(BF16)
        return pltpu.bitcast(wa, U32), pltpu.bitcast(wb, U32)

    def prep_scale(bn, j, rq, rk):
        mq = jnp.max(rq, axis=1, keepdims=True) + 2.0 ** -100
        mk = jnp.max(rk, axis=1, keepdims=True) + 2.0 ** -100
        b2 = jnp.broadcast_to(mq * mk, (8, 128))
        p2 = jnp.full((8, 128), 2.0 ** XMAX, F32)
        up = jnp.full((8, 128), 2.0 ** (2 ** XMAX), F32)
        for x in reversed(range(XMAX)):
            ok = b2 <= (MARGIN * 2.0 ** (x - 1)) ** 2
            p2 = jnp.where(ok, 2.0 ** x, p2)
            up = jnp.where(ok, 2.0 ** (2 ** x), up)
        fast = jnp.where(b2 <= (MARGIN * 2.0 ** (XMAX - 1)) ** 2, 1, 0).astype(I32)
        consts = const_rows(p2)
        up_ref[bn & 1, j] = up
        cw_ref[bn & 1, j, 0] = consts[0]
        cw_ref[bn & 1, j, 1] = consts[1]
        return consts, fast

    def packed_dot(kc, wq, consts):
        w = jnp.concatenate([wq, tile4(consts[0]), wq, tile4(consts[1])], axis=0)
        return jnp.dot(pltpu.bitcast(kc, BF16), pltpu.bitcast(w, BF16),
                       preferred_element_type=F32)

    def qk(slot, j, tile, ci, consts):
        return packed_dot(kt_ref[slot, j, pl.ds(ci * 32, 32), :],
                          w_ref[slot, j, tile], consts)

    def decode(tt):
        hi = pltpu.bitcast(pltpu.bitcast(tt, U32) & jnp.uint32(0xFFFFF000), F32)
        return hi, (tt - hi) * (1.0 / EPS)

    def exp_chunk(tt, lh, ll):
        hi, lo = decode(tt)
        ph, plo = jnp.exp2(hi), jnp.exp2(lo)
        grp = [None] * ng
        for i in range(ng // 2):
            a = ph[16 * i:16 * i + 8] + ph[16 * i + 8:16 * i + 16]
            b = plo[16 * i:16 * i + 8] + plo[16 * i + 8:16 * i + 16]
            lh = a if lh is None else lh + a
            ll = b if ll is None else ll + b
            grp[ng - 1 - 2 * i] = ph[16 * i:16 * i + 16]
            grp[ng - 2 - 2 * i] = plo[16 * i:16 * i + 16]
        return jnp.concatenate(grp, axis=0).astype(BF16), lh, ll

    def store_carry(tt0):
        lh = ll = None
        for e in range(2):
            p, lh, ll = exp_chunk(tt0[e], lh, ll)
            p0_ref[e] = p
        l0_ref[0] = lh
        l0_ref[1] = ll

    def full_prep(bn):
        allfast = None
        for j in range(HB):
            rq = rk = None
            for i in range(nc):
                rq = prep_q(bn, j, i, rq)
            for ci in range(nc):
                rk = prep_k(bn, j, ci, rk)
            consts, fast = prep_scale(bn, j, rq, rk)
            if j == 0:
                store_carry([qk(bn & 1, 0, 0, e, consts) for e in range(2)])
            allfast = fast if allfast is None else allfast * fast
        return allfast[0, 0]

    def probe():
        r = lax.broadcasted_iota(I32, (D, tk), 0)
        cc = lax.broadcasted_iota(I32, (D, tk), 1)
        ks = (((r * 37 + cc * 11) & 127) - 63).astype(F32) * (2.0 ** -9)
        r = lax.broadcasted_iota(I32, (D, tq), 0)
        cc = lax.broadcasted_iota(I32, (D, tq), 1)
        qs = ((((r * 29 + cc * 13) & 127) - 63).astype(F32) * (2.0 ** -10)).astype(BF16)
        kc = jnp.concatenate(pack_lhs(ks), axis=0)
        tt = packed_dot(kc, pltpu.bitcast(qs, U32), const_rows(jnp.ones((8, 128), F32)))
        hi, lo = decode(tt)
        ex = lax.dot_general(ks.astype(BF16), qs, (((0,), (0,)), ((), ())),
                             preferred_element_type=F32)
        err = None
        for i in range(ng // 2):
            hi_g, lo_g = ng - 1 - 2 * i, ng - 2 - 2 * i
            e1 = jnp.abs(hi[16 * i:16 * i + 16] + 1.5 - ex[16 * hi_g:16 * hi_g + 16])
            e2 = jnp.abs(lo[16 * i:16 * i + 16] + 0.5 - ex[16 * lo_g:16 * lo_g + 16])
            e = jnp.maximum(e1, e2)
            err = e if err is None else jnp.maximum(err, e)
        bad = jnp.where(err <= 2.0 ** -11, 0.0, 1.0)
        return jnp.where(jnp.max(bad) == 0.0, 1, 0).astype(I32)

    def exact_block(b):
        prefetch(b)
        cur = b & 1
        n_tiles = HB * nq
        always = tile4(up_ref[cur, 0]) > 0.0
        for j in range(HB):
            for ci in range(nc):
                kr_ref[j, pl.ds(ci * 64, 64), :] = pltpu.bitcast(
                    kb_ref[b & 3, j, :, pl.ds(ci * tk, tk)].T, U32)

        def stage(it_qk, it_pv, m):
            if it_qk is not None:
                jq = it_qk // nq
                wq = pltpu.bitcast(w_ref[cur, jq, it_qk % nq], BF16)
            if it_pv is not None:
                jv = it_pv // nq
            m8 = l8 = acc = prev = None
            for ci in range(nc):
                if it_pv is not None:
                    s_cur = s_ref[pl.ds(ci * tk, tk), :]
                cm = None
                if it_qk is not None:
                    kc = pltpu.bitcast(kr_ref[jq, pl.ds(ci * 64, 64), :], BF16)
                    s = jnp.dot(kc, wq, preferred_element_type=F32)
                    s_ref[pl.ds(ci * tk, tk), :] = s
                    cm = [jnp.maximum(s[16 * r:16 * r + 8], s[16 * r + 8:16 * r + 16])
                          for r in range(ng)]
                    for a in cm:
                        m8 = a if m8 is None else jnp.maximum(m8, a)
                if it_pv is not None:
                    ps = [None] * ng
                    for i, r in enumerate(reversed(range(ng))):
                        if i % 2 == 0:
                            mg = m if prev is None else jnp.where(always, m, prev[i])
                        pa = jnp.exp2((s_cur[16 * r:16 * r + 8] - mg) * c)
                        pb = jnp.exp2((s_cur[16 * r + 8:16 * r + 16] - mg) * c)
                        l8 = pa + pb if l8 is None else l8 + (pa + pb)
                        ps[r] = jnp.concatenate([pa, pb], axis=0)
                    p = jnp.concatenate(ps, axis=0).astype(BF16)
                    pv = jnp.dot(vb_ref[cur, jv, :, pl.ds(ci * tk, tk)], p,
                                 preferred_element_type=F32)
                    acc = pv if acc is None else acc + pv
                prev = cm
            if it_pv is not None:
                l = jnp.sum(l8, axis=0, keepdims=True)
                off = pl.multiple_of((it_pv % nq) * tq, tq)
                ob_ref[cur, jv, :, pl.ds(off, tq)] = (acc * (1.0 / l)).astype(ob_ref.dtype)
            if it_qk is None:
                return None
            return jnp.broadcast_to(jnp.max(m8, axis=0, keepdims=True), (8, tq))

        m = stage(0, None, None)
        m = lax.fori_loop(0, n_tiles - 1, lambda i, mm: stage(i + 1, i, mm), m)
        for j in range(HB - 1):
            o_copy(b, j).start()
        stage(None, n_tiles - 1, m)
        return full_prep(b + 1)

    def packed_block(b):
        cur = b & 1
        bn = b + 1
        consts = [(cw_ref[cur, j, 0], cw_ref[cur, j, 1]) for j in range(HB)]
        ups = [up_ref[cur, j] for j in range(HB)]
        lane = lax.broadcasted_iota(I32, (8, tk), 1)
        odd = (lane // 16) % 2 == 1

        always = ups[0] > 0.0
        ties = {}

        def tie(e, val):
            if val.dtype != U32:
                val = pltpu.bitcast(jnp.broadcast_to(val, (8, 128)), U32)
            ties.setdefault(e, []).append(val)

        def prep_v(j, ci, e_tie):
            upv = jnp.where(odd, ups[j], 1.0)
            vf = vb_ref[cur, j, :, pl.ds(ci * tk, tk)].astype(F32)
            vf = (vf.reshape(D // 8, 8, tk) * upv[None]).reshape(D, tk)
            vhu = pltpu.bitcast(vf.astype(BF16), U32)
            vh_ref[cur, j, :, pl.ds(ci * tk, tk)] = vhu
            if e_tie is not None:
                tie(e_tie, vhu[0:8])
                tie(e_tie, vhu[8:16])

        per_head = nq * nc
        n_steps = HB * per_head
        tts, tt0, runs = {}, [], []
        lh = ll = acc = rq = rk = allfast = nconsts0 = None
        for e in range(n_steps):
            j, el = divmod(e, per_head)
            tile, ci = divmod(el, nc)
            if e + 2 < n_steps:
                j1, el1 = divmod(e + 2, per_head)
                t1, c1 = divmod(el1, nc)
                cb = consts[j1][1]
                vals = ties.pop(e + 2, [])
                if vals:
                    cb = jnp.where(always, cb, functools.reduce(jnp.bitwise_or, vals))
                tts[e + 2] = qk(cur, j1, t1, c1, (consts[j1][0], cb))
            else:
                tt0.append(qk(bn & 1, 0, 0, e + 2 - n_steps, nconsts0))
            if e == 0:
                prefetch(b)
                for cv in range(nc):
                    et = V_TIE + cv // V_PROG
                    prep_v(0, cv, et if et < cv + 2 else None)
            if j >= 1 and el == 8:
                o_copy(b, j - 1).start()
            jp = (j + 1) % HB
            if el == 0:
                rq = rk = None
            if (el - Q0) % QSTEP == 0 and 0 <= (el - Q0) // QSTEP < nc:
                rq = prep_q(bn, jp, (el - Q0) // QSTEP, rq)
                tie(e + TIE_LAG, rq)
            if (el - K0) % KSTEP == 0 and 0 <= (el - K0) // KSTEP < nc:
                rk = prep_k(bn, jp, (el - K0) // KSTEP, rk)
                tie(e + TIE_LAG, rk)
            if j + 1 < HB and (el - V0) % VSTEP == 0 and 0 <= (el - V0) // VSTEP < nc:
                prep_v(j + 1, (el - V0) // VSTEP, e + TIE_LAG)
            if el == FIN:
                runs.append((jp, rq, rk))
                if j == HB - 1:
                    for jn, rqn, rkn in runs:
                        nconsts, fast = prep_scale(bn, jn, rqn, rkn)
                        tie(e + TIE_LAG, nconsts[0])
                        tie(e + TIE_LAG, nconsts[1])
                        if jn == 0:
                            nconsts0 = nconsts
                        allfast = fast if allfast is None else allfast * fast
            if ci == 0:
                lh = ll = None
            if e == 0:
                lh, ll = l0_ref[0], l0_ref[1]
            if e < 2:
                p = p0_ref[e]
            else:
                p, lh, ll = exp_chunk(tts.pop(e), lh, ll)
            vh = pltpu.bitcast(vh_ref[cur, j, :, pl.ds(ci * tk, tk)], BF16)
            pv = jnp.dot(vh, p, preferred_element_type=F32)
            acc = pv if ci == 0 else acc + pv
            if ci == nc - 1:
                l = jnp.sum(lh * tile4(ups[j]) + ll, axis=0, keepdims=True)
                r0 = pl.reciprocal(l, approx=True)
                rinv = r0 * (2.0 - l * r0)
                of = acc * rinv
                for u in range(tq // 128):
                    tie(e + R_TIE, rinv[:, u * 128:(u + 1) * 128])
                    tie(e + O_TIE, of[D - 8:D, u * 128:(u + 1) * 128])
                ob_ref[cur, j, :, tile * tq:(tile + 1) * tq] = of.astype(ob_ref.dtype)
        store_carry(tt0)
        return allfast[0, 0]

    zero = jnp.int32(0)
    q_copy(zero).start()
    k_copy(zero).start()
    v_copy(zero).start()
    q_copy(zero + 1).start()
    k_copy(zero + 1).start()
    ok = probe()
    q_copy(zero).wait()
    k_copy(zero).wait()
    fast0 = full_prep(zero) * ok

    def body(b, fast):
        @pl.when(b >= 1)
        def _():
            o_copy(b - 1, HB - 1).start()

        v_copy(b).wait()
        q_copy(b + 1).wait()
        k_copy(b + 1).wait()

        @pl.when(b >= 2)
        def _():
            for j in range(HB):
                o_copy(b - 2, j).wait()

        return lax.cond(fast == 1, packed_block, exact_block, b) * ok

    lax.fori_loop(0, NB, body, fast0)
    last = jnp.int32(NB)
    o_copy(last - 1, HB - 1).start()
    v_copy(last).wait()
    q_copy(last + 1).wait()
    k_copy(last + 1).wait()
    for j in range(HB):
        o_copy(last - 2, j).wait()
        o_copy(last - 1, j).wait()


@jax.jit
def pallas_standalone__fused_io_aware_attn__prompt_kernel(
    q: jax.Array,
    k: jax.Array,
    v: jax.Array,
):
    B, H, S, D = q.shape
    NB = B * H // HB
    qT, kT, vT = (jnp.swapaxes(x, -1, -2).reshape(NB, HB, D, S) for x in (q, k, v))
    hbm = pl.BlockSpec(memory_space=pl.ANY)
    oT = pl.pallas_call(
        _attn_kernel,
        in_specs=[hbm, hbm, hbm],
        out_specs=hbm,
        out_shape=jax.ShapeDtypeStruct((NB, HB, D, S), q.dtype),
        scratch_shapes=[
            pltpu.VMEM((2, HB, D, S), BF16),
            pltpu.VMEM((4, HB, D, S), BF16),
            pltpu.VMEM((2, HB, D, S), BF16),
            pltpu.VMEM((2, HB, D, S), BF16),
            pltpu.SemaphoreType.DMA((3 + HB, 2)),
            pltpu.VMEM((2, HB, S // 4, KA), U32),
            pltpu.VMEM((2, HB, S // TQ, D // 2, TQ), U32),
            pltpu.VMEM((2, HB, D // 2, S), U32),
            pltpu.VMEM((2, TK, TQ), BF16),
            pltpu.VMEM((2, 8, TQ), F32),
            pltpu.VMEM((2, HB, 8, 128), F32),
            pltpu.VMEM((2, HB, 2, 8, 128), U32),
            pltpu.VMEM((S, TQ), F32),
            pltpu.VMEM((HB, S // 2, D), U32),
        ],
        compiler_params=pltpu.CompilerParams(
            disable_bounds_checks=True,
            vmem_limit_bytes=64 * 1024 * 1024),
    )(qT, kT, vT)
    return jnp.swapaxes(oT.reshape(B, H, D, S), -1, -2)
```

```python
import functools
import math

import jax
import jax.numpy as jnp
from jax import lax
import jax.experimental.pallas as pl
import jax.experimental.pallas.tpu as pltpu

F32, BF16, U32, I32 = jnp.float32, jnp.bfloat16, jnp.uint32, jnp.int32

HB = 2
TQ = 512
TK = 128
KA = 96
EPS = 2.0 ** -11
XMAX = 4
MARGIN = 0.97

Q0, QSTEP, K0, KSTEP, V0, VSTEP, FIN = 14, 1, 10, 3, 8, 3, 58
TIE_LAG, V_TIE, V_PROG, R_TIE, O_TIE = 3, 3, 2, 4, 6


def _attn_kernel(q_hbm, k_hbm, v_hbm, o_hbm,
                 qb_ref, kb_ref, vb_ref, ob_ref, sem,
                 kt_ref, w_ref, vh_ref, p0_ref, l0_ref, up_ref, cw_ref,
                 s_ref, kr_ref):
    NB, _, D, S = q_hbm.shape
    tq, tk = TQ, TK
    c = (D ** -0.5) * math.log2(math.e)
    nq = S // tq
    nc = S // tk
    ng = tk // 16
    lo0 = D + 16

    def tile4(z):
        return jnp.concatenate([z] * (tq // 128), axis=1)

    def q_copy(b):
        return pltpu.make_async_copy(
            q_hbm.at[jnp.minimum(b, NB - 1)], qb_ref.at[b & 1], sem.at[0, b & 1])

    def k_copy(b):
        return pltpu.make_async_copy(
            k_hbm.at[jnp.minimum(b, NB - 1)], kb_ref.at[b & 3], sem.at[1, b & 1])

    def v_copy(b):
        return pltpu.make_async_copy(
            v_hbm.at[jnp.minimum(b, NB - 1)], vb_ref.at[b & 1], sem.at[2, b & 1])

    def o_copy(b, j):
        return pltpu.make_async_copy(
            ob_ref.at[b & 1, j], o_hbm.at[b, j], sem.at[3 + j, b & 1])

    def prefetch(b):
        v_copy(b + 1).start()
        q_copy(b + 2).start()
        k_copy(b + 2).start()

    def pack_lhs(ks):
        row = lax.broadcasted_iota(I32, (8, tk), 0)
        lane = lax.broadcasted_iota(I32, (8, KA), 1)
        e0 = jnp.where(row == 0, 1.0, 0.0)
        e01 = jnp.where(row < 2, 1.0, 0.0)
        aug = jnp.concatenate(
            [ks, e0, e0, ks * EPS, e01, jnp.zeros_like(e0)], axis=0).astype(BF16)
        z = pltpu.bitcast(aug.T, U32)
        out = []
        for i in range(ng // 2):
            hi_g, lo_g = ng - 1 - 2 * i, ng - 2 - 2 * i
            out.append(jnp.where(lane < lo0, z[8 * hi_g:8 * hi_g + 8],
                                 z[8 * lo_g:8 * lo_g + 8]))
        return out

    def prep_k(bn, j, ci, run):
        ks = kb_ref[bn & 3, j, :, pl.ds(ci * tk, tk)].astype(F32) * c
        for i, zz in enumerate(pack_lhs(ks)):
            kt_ref[bn & 1, j, pl.ds(ci * 32 + 8 * i, 8), :] = zz
        n2 = jnp.sum(ks * ks, axis=0, keepdims=True)
        return n2 if run is None else jnp.maximum(run, n2)

    def prep_q(bn, j, i, run):
        qb = qb_ref[bn & 1, j, :, i * 128:(i + 1) * 128]
        ti, off = divmod(i * 128, tq)
        w_ref[bn & 1, j, ti, :, off:off + 128] = pltpu.bitcast(qb, U32)
        x = qb.astype(F32)
        n2 = jnp.sum(x * x, axis=0, keepdims=True)
        return n2 if run is None else jnp.maximum(run, n2)

    def const_rows(p2):
        row = lax.broadcasted_iota(I32, (8, 128), 0)
        a0 = jnp.where(row == 0, 1.5 * 2.0 ** 12, 0.0) * p2
        b0 = jnp.where(row == 0, -1.5, jnp.where(row == 1, -(2.0 ** -12), 0.0)) * p2
        wa = jnp.concatenate([a0, -a0], axis=0).astype(BF16)
        wb = jnp.concatenate([b0, jnp.zeros_like(b0)], axis=0).astype(BF16)
        return pltpu.bitcast(wa, U32), pltpu.bitcast(wb, U32)

    def prep_scale(bn, j, rq, rk):
        mq = jnp.max(rq, axis=1, keepdims=True) + 2.0 ** -100
        mk = jnp.max(rk, axis=1, keepdims=True) + 2.0 ** -100
        b2 = jnp.broadcast_to(mq * mk, (8, 128))
        p2 = jnp.full((8, 128), 2.0 ** XMAX, F32)
        up = jnp.full((8, 128), 2.0 ** (2 ** XMAX), F32)
        for x in reversed(range(XMAX)):
            ok = b2 <= (MARGIN * 2.0 ** (x - 1)) ** 2
            p2 = jnp.where(ok, 2.0 ** x, p2)
            up = jnp.where(ok, 2.0 ** (2 ** x), up)
        fast = jnp.where(b2 <= (MARGIN * 2.0 ** (XMAX - 1)) ** 2, 1, 0).astype(I32)
        consts = const_rows(p2)
        up_ref[bn & 1, j] = up
        cw_ref[bn & 1, j, 0] = consts[0]
        cw_ref[bn & 1, j, 1] = consts[1]
        return consts, fast

    def packed_dot(kc, wq, consts):
        w = jnp.concatenate([wq, tile4(consts[0]), wq, tile4(consts[1])], axis=0)
        return jnp.dot(pltpu.bitcast(kc, BF16), pltpu.bitcast(w, BF16),
                       preferred_element_type=F32)

    def qk(slot, j, tile, ci, consts):
        return packed_dot(kt_ref[slot, j, pl.ds(ci * 32, 32), :],
                          w_ref[slot, j, tile], consts)

    def decode(tt):
        hi = pltpu.bitcast(pltpu.bitcast(tt, U32) & jnp.uint32(0xFFFFF000), F32)
        return hi, (tt - hi) * (1.0 / EPS)

    def exp_chunk(tt, lh, ll):
        hi, lo = decode(tt)
        ph, plo = jnp.exp2(hi), jnp.exp2(lo)
        grp = [None] * ng
        for i in range(ng // 2):
            a = ph[16 * i:16 * i + 8] + ph[16 * i + 8:16 * i + 16]
            b = plo[16 * i:16 * i + 8] + plo[16 * i + 8:16 * i + 16]
            lh = a if lh is None else lh + a
            ll = b if ll is None else ll + b
            grp[ng - 1 - 2 * i] = ph[16 * i:16 * i + 16]
            grp[ng - 2 - 2 * i] = plo[16 * i:16 * i + 16]
        return jnp.concatenate(grp, axis=0).astype(BF16), lh, ll

    def store_carry(tt0):
        lh = ll = None
        for e in range(2):
            p, lh, ll = exp_chunk(tt0[e], lh, ll)
            p0_ref[e] = p
        l0_ref[0] = lh
        l0_ref[1] = ll

    def full_prep(bn):
        allfast = None
        for j in range(HB):
            rq = rk = None
            for i in range(nc):
                rq = prep_q(bn, j, i, rq)
            for ci in range(nc):
                rk = prep_k(bn, j, ci, rk)
            consts, fast = prep_scale(bn, j, rq, rk)
            if j == 0:
                store_carry([qk(bn & 1, 0, 0, e, consts) for e in range(2)])
            allfast = fast if allfast is None else allfast * fast
        return allfast[0, 0]

    def probe():
        r = lax.broadcasted_iota(I32, (D, tk), 0)
        cc = lax.broadcasted_iota(I32, (D, tk), 1)
        ks = (((r * 37 + cc * 11) & 127) - 63).astype(F32) * (2.0 ** -9)
        r = lax.broadcasted_iota(I32, (D, tq), 0)
        cc = lax.broadcasted_iota(I32, (D, tq), 1)
        qs = ((((r * 29 + cc * 13) & 127) - 63).astype(F32) * (2.0 ** -10)).astype(BF16)
        kc = jnp.concatenate(pack_lhs(ks), axis=0)
        tt = packed_dot(kc, pltpu.bitcast(qs, U32), const_rows(jnp.ones((8, 128), F32)))
        hi, lo = decode(tt)
        ex = lax.dot_general(ks.astype(BF16), qs, (((0,), (0,)), ((), ())),
                             preferred_element_type=F32)
        err = None
        for i in range(ng // 2):
            hi_g, lo_g = ng - 1 - 2 * i, ng - 2 - 2 * i
            e1 = jnp.abs(hi[16 * i:16 * i + 16] + 1.5 - ex[16 * hi_g:16 * hi_g + 16])
            e2 = jnp.abs(lo[16 * i:16 * i + 16] + 0.5 - ex[16 * lo_g:16 * lo_g + 16])
            e = jnp.maximum(e1, e2)
            err = e if err is None else jnp.maximum(err, e)
        bad = jnp.where(err <= 2.0 ** -11, 0.0, 1.0)
        return jnp.where(jnp.max(bad) == 0.0, 1, 0).astype(I32)

    def exact_block(b):
        prefetch(b)
        cur = b & 1
        n_tiles = HB * nq
        always = tile4(up_ref[cur, 0]) > 0.0
        for j in range(HB):
            for ci in range(nc):
                kr_ref[j, pl.ds(ci * 64, 64), :] = pltpu.bitcast(
                    kb_ref[b & 3, j, :, pl.ds(ci * tk, tk)].T, U32)

        def stage(it_qk, it_pv, m):
            if it_qk is not None:
                jq = it_qk // nq
                wq = pltpu.bitcast(w_ref[cur, jq, it_qk % nq], BF16)
            if it_pv is not None:
                jv = it_pv // nq
            m8 = l8 = acc = prev = None
            for ci in range(nc):
                if it_pv is not None:
                    s_cur = s_ref[pl.ds(ci * tk, tk), :]
                cm = None
                if it_qk is not None:
                    kc = pltpu.bitcast(kr_ref[jq, pl.ds(ci * 64, 64), :], BF16)
                    s = jnp.dot(kc, wq, preferred_element_type=F32)
                    s_ref[pl.ds(ci * tk, tk), :] = s
                    cm = [jnp.maximum(s[16 * r:16 * r + 8], s[16 * r + 8:16 * r + 16])
                          for r in range(ng)]
                    for a in cm:
                        m8 = a if m8 is None else jnp.maximum(m8, a)
                if it_pv is not None:
                    ps = [None] * ng
                    for i, r in enumerate(reversed(range(ng))):
                        if i % 2 == 0:
                            mg = m if prev is None else jnp.where(always, m, prev[i])
                        pa = jnp.exp2((s_cur[16 * r:16 * r + 8] - mg) * c)
                        pb = jnp.exp2((s_cur[16 * r + 8:16 * r + 16] - mg) * c)
                        l8 = pa + pb if l8 is None else l8 + (pa + pb)
                        ps[r] = jnp.concatenate([pa, pb], axis=0)
                    p = jnp.concatenate(ps, axis=0).astype(BF16)
                    pv = jnp.dot(vb_ref[cur, jv, :, pl.ds(ci * tk, tk)], p,
                                 preferred_element_type=F32)
                    acc = pv if acc is None else acc + pv
                prev = cm
            if it_pv is not None:
                l = jnp.sum(l8, axis=0, keepdims=True)
                off = pl.multiple_of((it_pv % nq) * tq, tq)
                ob_ref[cur, jv, :, pl.ds(off, tq)] = (acc * (1.0 / l)).astype(ob_ref.dtype)
            if it_qk is None:
                return None
            return jnp.broadcast_to(jnp.max(m8, axis=0, keepdims=True), (8, tq))

        m = stage(0, None, None)
        m = lax.fori_loop(0, n_tiles - 1, lambda i, mm: stage(i + 1, i, mm), m)
        for j in range(HB - 1):
            o_copy(b, j).start()
        stage(None, n_tiles - 1, m)
        return full_prep(b + 1)

    def packed_block(b):
        cur = b & 1
        bn = b + 1
        consts = [(cw_ref[cur, j, 0], cw_ref[cur, j, 1]) for j in range(HB)]
        ups = [up_ref[cur, j] for j in range(HB)]
        lane = lax.broadcasted_iota(I32, (8, tk), 1)
        odd = (lane // 16) % 2 == 1

        always = ups[0] > 0.0
        ties = {}

        def tie(e, val):
            if val.dtype != U32:
                val = pltpu.bitcast(jnp.broadcast_to(val, (8, 128)), U32)
            ties.setdefault(e, []).append(val)

        def prep_v(j, ci, e_tie):
            upv = jnp.where(odd, ups[j], 1.0)
            vf = vb_ref[cur, j, :, pl.ds(ci * tk, tk)].astype(F32)
            vf = (vf.reshape(D // 8, 8, tk) * upv[None]).reshape(D, tk)
            vhu = pltpu.bitcast(vf.astype(BF16), U32)
            vh_ref[cur, j, :, pl.ds(ci * tk, tk)] = vhu
            if e_tie is not None:
                tie(e_tie, vhu[0:8])
                tie(e_tie, vhu[8:16])

        per_head = nq * nc
        n_steps = HB * per_head
        tts, tt0, runs = {}, [], []
        lh = ll = acc = rq = rk = allfast = nconsts0 = None
        for e in range(n_steps):
            j, el = divmod(e, per_head)
            tile, ci = divmod(el, nc)
            if e + 2 < n_steps:
                j1, el1 = divmod(e + 2, per_head)
                t1, c1 = divmod(el1, nc)
                cb = consts[j1][1]
                vals = ties.pop(e + 2, [])
                if vals:
                    cb = jnp.where(always, cb, functools.reduce(jnp.bitwise_or, vals))
                tts[e + 2] = qk(cur, j1, t1, c1, (consts[j1][0], cb))
            else:
                tt0.append(qk(bn & 1, 0, 0, e + 2 - n_steps, nconsts0))
            if e == 0:
                prefetch(b)
                for cv in range(nc):
                    et = V_TIE + cv // V_PROG
                    prep_v(0, cv, et if et < cv + 2 else None)
            if j >= 1 and el == 8:
                o_copy(b, j - 1).start()
            jp = (j + 1) % HB
            if el == 0:
                rq = rk = None
            if (el - Q0) % QSTEP == 0 and 0 <= (el - Q0) // QSTEP < nc:
                rq = prep_q(bn, jp, (el - Q0) // QSTEP, rq)
                tie(e + TIE_LAG, rq)
            if (el - K0) % KSTEP == 0 and 0 <= (el - K0) // KSTEP < nc:
                rk = prep_k(bn, jp, (el - K0) // KSTEP, rk)
                tie(e + TIE_LAG, rk)
            if j + 1 < HB and (el - V0) % VSTEP == 0 and 0 <= (el - V0) // VSTEP < nc:
                prep_v(j + 1, (el - V0) // VSTEP, e + TIE_LAG)
            if el == FIN:
                runs.append((jp, rq, rk))
                if j == HB - 1:
                    for jn, rqn, rkn in runs:
                        nconsts, fast = prep_scale(bn, jn, rqn, rkn)
                        tie(e + TIE_LAG, nconsts[0])
                        tie(e + TIE_LAG, nconsts[1])
                        if jn == 0:
                            nconsts0 = nconsts
                        allfast = fast if allfast is None else allfast * fast
            if ci == 0:
                lh = ll = None
            if e == 0:
                lh, ll = l0_ref[0], l0_ref[1]
            if e < 2:
                p = p0_ref[e]
            else:
                p, lh, ll = exp_chunk(tts.pop(e), lh, ll)
            vh = pltpu.bitcast(vh_ref[cur, j, :, pl.ds(ci * tk, tk)], BF16)
            pv = jnp.dot(vh, p, preferred_element_type=F32)
            acc = pv if ci == 0 else acc + pv
            if ci == nc - 1:
                l = jnp.sum(lh * tile4(ups[j]) + ll, axis=0, keepdims=True)
                r0 = pl.reciprocal(l, approx=True)
                rinv = r0 * (2.0 - l * r0)
                of = acc * rinv
                for u in range(tq // 128):
                    tie(e + R_TIE, rinv[:, u * 128:(u + 1) * 128])
                    tie(e + O_TIE, of[D - 8:D, u * 128:(u + 1) * 128])
                ob_ref[cur, j, :, tile * tq:(tile + 1) * tq] = of.astype(ob_ref.dtype)
        store_carry(tt0)
        return allfast[0, 0]

    zero = jnp.int32(0)
    q_copy(zero).start()
    k_copy(zero).start()
    prefetch(zero - 1)
    ok = probe()
    q_copy(zero).wait()
    k_copy(zero).wait()
    fast0 = full_prep(zero) * ok

    def body(b, fast):
        @pl.when(b >= 1)
        def _():
            o_copy(b - 1, HB - 1).start()

        v_copy(b).wait()
        q_copy(b + 1).wait()
        k_copy(b + 1).wait()

        @pl.when(b >= 2)
        def _():
            for j in range(HB):
                o_copy(b - 2, j).wait()

        return lax.cond(fast == 1, packed_block, exact_block, b) * ok

    lax.fori_loop(0, NB, body, fast0)
    last = jnp.int32(NB)
    o_copy(last - 1, HB - 1).start()
    v_copy(last).wait()
    q_copy(last + 1).wait()
    k_copy(last + 1).wait()
    for j in range(HB):
        o_copy(last - 2, j).wait()
        o_copy(last - 1, j).wait()


@jax.jit
def pallas_standalone__fused_io_aware_attn__prompt_kernel(
    q: jax.Array,
    k: jax.Array,
    v: jax.Array,
):
    B, H, S, D = q.shape
    NB = B * H // HB
    qT, kT, vT = (jnp.swapaxes(x, -1, -2).reshape(NB, HB, D, S) for x in (q, k, v))
    hbm = pl.BlockSpec(memory_space=pl.ANY)
    oT = pl.pallas_call(
        _attn_kernel,
        in_specs=[hbm, hbm, hbm],
        out_specs=hbm,
        out_shape=jax.ShapeDtypeStruct((NB, HB, D, S), q.dtype),
        scratch_shapes=[
            pltpu.VMEM((2, HB, D, S), BF16),
            pltpu.VMEM((4, HB, D, S), BF16),
            pltpu.VMEM((2, HB, D, S), BF16),
            pltpu.VMEM((2, HB, D, S), BF16),
            pltpu.SemaphoreType.DMA((3 + HB, 2)),
            pltpu.VMEM((2, HB, S // 4, KA), U32),
            pltpu.VMEM((2, HB, S // TQ, D // 2, TQ), U32),
            pltpu.VMEM((2, HB, D // 2, S), U32),
            pltpu.VMEM((2, TK, TQ), BF16),
            pltpu.VMEM((2, 8, TQ), F32),
            pltpu.VMEM((2, HB, 8, 128), F32),
            pltpu.VMEM((2, HB, 2, 8, 128), U32),
            pltpu.VMEM((S, TQ), F32),
            pltpu.VMEM((HB, S // 2, D), U32),
        ],
        compiler_params=pltpu.CompilerParams(
            disable_bounds_checks=True,
            vmem_limit_bytes=64 * 1024 * 1024),
    )(qT, kT, vT)
    return jnp.swapaxes(oT.reshape(B, H, D, S), -1, -2)
```

```python
import functools
import math

import jax
import jax.numpy as jnp
from jax import lax
import jax.experimental.pallas as pl
import jax.experimental.pallas.tpu as pltpu

F32, BF16, U32, I32 = jnp.float32, jnp.bfloat16, jnp.uint32, jnp.int32

HB = 2
TQ = 512
TK = 128
KA = 96
EPS = 2.0 ** -11
XMAX = 4
MARGIN = 0.97

Q0, QSTEP, K0, KSTEP, V0, VSTEP, FIN = 14, 1, 10, 3, 8, 3, 58
TIE_LAG, V_TIE, V_PROG, R_TIE, O_TIE = 3, 3, 2, 4, 6


def _attn_kernel(q_hbm, k_hbm, v_hbm, o_hbm,
                 qb_ref, kb_ref, vb_ref, ob_ref, sem,
                 kt_ref, w_ref, vh_ref, p0_ref, l0_ref, up_ref, cw_ref,
                 s_ref, kr_ref):
    NB, _, D, S = q_hbm.shape
    tq, tk = TQ, TK
    c = (D ** -0.5) * math.log2(math.e)
    nq = S // tq
    nc = S // tk
    ng = tk // 16
    lo0 = D + 16

    def tile4(z):
        return jnp.concatenate([z] * (tq // 128), axis=1)

    def q_copy(b):
        return pltpu.make_async_copy(
            q_hbm.at[jnp.minimum(b, NB - 1)], qb_ref.at[b & 1], sem.at[0])

    def k_copy(b):
        return pltpu.make_async_copy(
            k_hbm.at[jnp.minimum(b, NB - 1)], kb_ref.at[b & 3], sem.at[1])

    def v_copy(b):
        return pltpu.make_async_copy(
            v_hbm.at[jnp.minimum(b, NB - 1)], vb_ref.at[b & 1], sem.at[2])

    def o_copy(b, j):
        return pltpu.make_async_copy(
            ob_ref.at[b & 1, j], o_hbm.at[b, j], sem.at[3 + j])

    def prefetch(b):
        @pl.when(b >= 1)
        def _():
            o_copy(b - 1, HB - 1).start()

        v_copy(b + 1).start()
        q_copy(b + 2).start()
        k_copy(b + 2).start()

    def pack_lhs(ks):
        row = lax.broadcasted_iota(I32, (8, tk), 0)
        lane = lax.broadcasted_iota(I32, (8, KA), 1)
        e0 = jnp.where(row == 0, 1.0, 0.0)
        e01 = jnp.where(row < 2, 1.0, 0.0)
        aug = jnp.concatenate(
            [ks, e0, e0, ks * EPS, e01, jnp.zeros_like(e0)], axis=0).astype(BF16)
        z = pltpu.bitcast(aug.T, U32)
        out = []
        for i in range(ng // 2):
            hi_g, lo_g = ng - 1 - 2 * i, ng - 2 - 2 * i
            out.append(jnp.where(lane < lo0, z[8 * hi_g:8 * hi_g + 8],
                                 z[8 * lo_g:8 * lo_g + 8]))
        return out

    def prep_k(bn, j, ci, run):
        ks = kb_ref[bn & 3, j, :, pl.ds(ci * tk, tk)].astype(F32) * c
        for i, zz in enumerate(pack_lhs(ks)):
            kt_ref[bn & 1, j, pl.ds(ci * 32 + 8 * i, 8), :] = zz
        n2 = jnp.sum(ks * ks, axis=0, keepdims=True)
        return n2 if run is None else jnp.maximum(run, n2)

    def prep_q(bn, j, i, run):
        qb = qb_ref[bn & 1, j, :, i * 128:(i + 1) * 128]
        ti, off = divmod(i * 128, tq)
        w_ref[bn & 1, j, ti, :, off:off + 128] = pltpu.bitcast(qb, U32)
        x = qb.astype(F32)
        n2 = jnp.sum(x * x, axis=0, keepdims=True)
        return n2 if run is None else jnp.maximum(run, n2)

    def const_rows(p2):
        row = lax.broadcasted_iota(I32, (8, 128), 0)
        a0 = jnp.where(row == 0, 1.5 * 2.0 ** 12, 0.0) * p2
        b0 = jnp.where(row == 0, -1.5, jnp.where(row == 1, -(2.0 ** -12), 0.0)) * p2
        wa = jnp.concatenate([a0, -a0], axis=0).astype(BF16)
        wb = jnp.concatenate([b0, jnp.zeros_like(b0)], axis=0).astype(BF16)
        return pltpu.bitcast(wa, U32), pltpu.bitcast(wb, U32)

    def prep_scale(bn, j, rq, rk):
        mq = jnp.max(rq, axis=1, keepdims=True) + 2.0 ** -100
        mk = jnp.max(rk, axis=1, keepdims=True) + 2.0 ** -100
        b2 = jnp.broadcast_to(mq * mk, (8, 128))
        p2 = jnp.full((8, 128), 2.0 ** XMAX, F32)
        up = jnp.full((8, 128), 2.0 ** (2 ** XMAX), F32)
        for x in reversed(range(XMAX)):
            ok = b2 <= (MARGIN * 2.0 ** (x - 1)) ** 2
            p2 = jnp.where(ok, 2.0 ** x, p2)
            up = jnp.where(ok, 2.0 ** (2 ** x), up)
        fast = jnp.where(b2 <= (MARGIN * 2.0 ** (XMAX - 1)) ** 2, 1, 0).astype(I32)
        consts = const_rows(p2)
        up_ref[bn & 1, j] = up
        cw_ref[bn & 1, j, 0] = consts[0]
        cw_ref[bn & 1, j, 1] = consts[1]
        return consts, fast

    def packed_dot(kc, wq, consts):
        w = jnp.concatenate([wq, tile4(consts[0]), wq, tile4(consts[1])], axis=0)
        return jnp.dot(pltpu.bitcast(kc, BF16), pltpu.bitcast(w, BF16),
                       preferred_element_type=F32)

    def qk(slot, j, tile, ci, consts):
        return packed_dot(kt_ref[slot, j, pl.ds(ci * 32, 32), :],
                          w_ref[slot, j, tile], consts)

    def decode(tt):
        hi = pltpu.bitcast(pltpu.bitcast(tt, U32) & jnp.uint32(0xFFFFF000), F32)
        return hi, (tt - hi) * (1.0 / EPS)

    def exp_chunk(tt, lh, ll):
        hi, lo = decode(tt)
        ph, plo = jnp.exp2(hi), jnp.exp2(lo)
        grp = [None] * ng
        for i in range(ng // 2):
            a = ph[16 * i:16 * i + 8] + ph[16 * i + 8:16 * i + 16]
            b = plo[16 * i:16 * i + 8] + plo[16 * i + 8:16 * i + 16]
            lh = a if lh is None else lh + a
            ll = b if ll is None else ll + b
            grp[ng - 1 - 2 * i] = ph[16 * i:16 * i + 16]
            grp[ng - 2 - 2 * i] = plo[16 * i:16 * i + 16]
        return jnp.concatenate(grp, axis=0).astype(BF16), lh, ll

    def store_carry(tt0):
        lh = ll = None
        for e in range(2):
            p, lh, ll = exp_chunk(tt0[e], lh, ll)
            p0_ref[e] = p
        l0_ref[0] = lh
        l0_ref[1] = ll

    def full_prep(bn):
        allfast = None
        for j in range(HB):
            rq = rk = None
            for i in range(nc):
                rq = prep_q(bn, j, i, rq)
            for ci in range(nc):
                rk = prep_k(bn, j, ci, rk)
            consts, fast = prep_scale(bn, j, rq, rk)
            if j == 0:
                store_carry([qk(bn & 1, 0, 0, e, consts) for e in range(2)])
            allfast = fast if allfast is None else allfast * fast
        return allfast[0, 0]

    def probe():
        r = lax.broadcasted_iota(I32, (D, tk), 0)
        cc = lax.broadcasted_iota(I32, (D, tk), 1)
        ks = (((r * 37 + cc * 11) & 127) - 63).astype(F32) * (2.0 ** -9)
        r = lax.broadcasted_iota(I32, (D, tq), 0)
        cc = lax.broadcasted_iota(I32, (D, tq), 1)
        qs = ((((r * 29 + cc * 13) & 127) - 63).astype(F32) * (2.0 ** -10)).astype(BF16)
        kc = jnp.concatenate(pack_lhs(ks), axis=0)
        tt = packed_dot(kc, pltpu.bitcast(qs, U32), const_rows(jnp.ones((8, 128), F32)))
        hi, lo = decode(tt)
        ex = lax.dot_general(ks.astype(BF16), qs, (((0,), (0,)), ((), ())),
                             preferred_element_type=F32)
        err = None
        for i in range(ng // 2):
            hi_g, lo_g = ng - 1 - 2 * i, ng - 2 - 2 * i
            e1 = jnp.abs(hi[16 * i:16 * i + 16] + 1.5 - ex[16 * hi_g:16 * hi_g + 16])
            e2 = jnp.abs(lo[16 * i:16 * i + 16] + 0.5 - ex[16 * lo_g:16 * lo_g + 16])
            e = jnp.maximum(e1, e2)
            err = e if err is None else jnp.maximum(err, e)
        bad = jnp.where(err <= 2.0 ** -11, 0.0, 1.0)
        return jnp.where(jnp.max(bad) == 0.0, 1, 0).astype(I32)

    def exact_block(b):
        prefetch(b)
        cur = b & 1
        n_tiles = HB * nq
        always = tile4(up_ref[cur, 0]) > 0.0
        for j in range(HB):
            for ci in range(nc):
                kr_ref[j, pl.ds(ci * 64, 64), :] = pltpu.bitcast(
                    kb_ref[b & 3, j, :, pl.ds(ci * tk, tk)].T, U32)

        def stage(it_qk, it_pv, m):
            if it_qk is not None:
                jq = it_qk // nq
                wq = pltpu.bitcast(w_ref[cur, jq, it_qk % nq], BF16)
            if it_pv is not None:
                jv = it_pv // nq
            m8 = l8 = acc = prev = None
            for ci in range(nc):
                if it_pv is not None:
                    s_cur = s_ref[pl.ds(ci * tk, tk), :]
                cm = None
                if it_qk is not None:
                    kc = pltpu.bitcast(kr_ref[jq, pl.ds(ci * 64, 64), :], BF16)
                    s = jnp.dot(kc, wq, preferred_element_type=F32)
                    s_ref[pl.ds(ci * tk, tk), :] = s
                    cm = [jnp.maximum(s[16 * r:16 * r + 8], s[16 * r + 8:16 * r + 16])
                          for r in range(ng)]
                    for a in cm:
                        m8 = a if m8 is None else jnp.maximum(m8, a)
                if it_pv is not None:
                    ps = [None] * ng
                    for i, r in enumerate(reversed(range(ng))):
                        if i % 2 == 0:
                            mg = m if prev is None else jnp.where(always, m, prev[i])
                        pa = jnp.exp2((s_cur[16 * r:16 * r + 8] - mg) * c)
                        pb = jnp.exp2((s_cur[16 * r + 8:16 * r + 16] - mg) * c)
                        l8 = pa + pb if l8 is None else l8 + (pa + pb)
                        ps[r] = jnp.concatenate([pa, pb], axis=0)
                    p = jnp.concatenate(ps, axis=0).astype(BF16)
                    pv = jnp.dot(vb_ref[cur, jv, :, pl.ds(ci * tk, tk)], p,
                                 preferred_element_type=F32)
                    acc = pv if acc is None else acc + pv
                prev = cm
            if it_pv is not None:
                l = jnp.sum(l8, axis=0, keepdims=True)
                off = pl.multiple_of((it_pv % nq) * tq, tq)
                ob_ref[cur, jv, :, pl.ds(off, tq)] = (acc * (1.0 / l)).astype(ob_ref.dtype)
            if it_qk is None:
                return None
            return jnp.broadcast_to(jnp.max(m8, axis=0, keepdims=True), (8, tq))

        m = stage(0, None, None)
        nfast = full_prep(b + 1)
        m = lax.fori_loop(0, n_tiles - 1, lambda i, mm: stage(i + 1, i, mm), m)
        for j in range(HB - 1):
            o_copy(b, j).start()
        stage(None, n_tiles - 1, m)
        return nfast

    def packed_block(b):
        cur = b & 1
        bn = b + 1
        consts = [(cw_ref[cur, j, 0], cw_ref[cur, j, 1]) for j in range(HB)]
        ups = [up_ref[cur, j] for j in range(HB)]
        lane = lax.broadcasted_iota(I32, (8, tk), 1)
        odd = (lane // 16) % 2 == 1

        always = ups[0] > 0.0
        ties = {}

        def tie(e, val):
            if val.dtype != U32:
                val = pltpu.bitcast(jnp.broadcast_to(val, (8, 128)), U32)
            ties.setdefault(e, []).append(val)

        def prep_v(j, ci, e_tie):
            upv = jnp.where(odd, ups[j], 1.0)
            vf = vb_ref[cur, j, :, pl.ds(ci * tk, tk)].astype(F32)
            vf = (vf.reshape(D // 8, 8, tk) * upv[None]).reshape(D, tk)
            vhu = pltpu.bitcast(vf.astype(BF16), U32)
            vh_ref[cur, j, :, pl.ds(ci * tk, tk)] = vhu
            if e_tie is not None:
                tie(e_tie, vhu[0:8])
                tie(e_tie, vhu[8:16])

        per_head = nq * nc
        n_steps = HB * per_head
        tts, tt0, runs = {}, [], []
        lh = ll = acc = rq = rk = allfast = nconsts0 = None
        for e in range(n_steps):
            j, el = divmod(e, per_head)
            tile, ci = divmod(el, nc)
            if e + 2 < n_steps:
                j1, el1 = divmod(e + 2, per_head)
                t1, c1 = divmod(el1, nc)
                cb = consts[j1][1]
                vals = ties.pop(e + 2, [])
                if vals:
                    cb = jnp.where(always, cb, functools.reduce(jnp.bitwise_or, vals))
                tts[e + 2] = qk(cur, j1, t1, c1, (consts[j1][0], cb))
            else:
                tt0.append(qk(bn & 1, 0, 0, e + 2 - n_steps, nconsts0))
            if e == 0:
                prefetch(b)
                for cv in range(nc):
                    et = V_TIE + cv // V_PROG
                    prep_v(0, cv, et if et < cv + 2 else None)
            if j >= 1 and el == 8:
                o_copy(b, j - 1).start()
            jp = (j + 1) % HB
            if el == 0:
                rq = rk = None
            if (el - Q0) % QSTEP == 0 and 0 <= (el - Q0) // QSTEP < nc:
                rq = prep_q(bn, jp, (el - Q0) // QSTEP, rq)
                tie(e + TIE_LAG, rq)
            if (el - K0) % KSTEP == 0 and 0 <= (el - K0) // KSTEP < nc:
                rk = prep_k(bn, jp, (el - K0) // KSTEP, rk)
                tie(e + TIE_LAG, rk)
            if j + 1 < HB and (el - V0) % VSTEP == 0 and 0 <= (el - V0) // VSTEP < nc:
                prep_v(j + 1, (el - V0) // VSTEP, e + TIE_LAG)
            if el == FIN:
                runs.append((jp, rq, rk))
                if j == HB - 1:
                    for jn, rqn, rkn in runs:
                        nconsts, fast = prep_scale(bn, jn, rqn, rkn)
                        tie(e + TIE_LAG, nconsts[0])
                        tie(e + TIE_LAG, nconsts[1])
                        if jn == 0:
                            nconsts0 = nconsts
                        allfast = fast if allfast is None else allfast * fast
            if ci == 0:
                lh = ll = None
            if e == 0:
                lh, ll = l0_ref[0], l0_ref[1]
            if e < 2:
                p = p0_ref[e]
            else:
                p, lh, ll = exp_chunk(tts.pop(e), lh, ll)
            vh = pltpu.bitcast(vh_ref[cur, j, :, pl.ds(ci * tk, tk)], BF16)
            pv = jnp.dot(vh, p, preferred_element_type=F32)
            acc = pv if ci == 0 else acc + pv
            if ci == nc - 1:
                l = jnp.sum(lh * tile4(ups[j]) + ll, axis=0, keepdims=True)
                r0 = pl.reciprocal(l, approx=True)
                rinv = r0 * (2.0 - l * r0)
                of = acc * rinv
                for u in range(tq // 128):
                    tie(e + R_TIE, rinv[:, u * 128:(u + 1) * 128])
                    tie(e + O_TIE, of[D - 8:D, u * 128:(u + 1) * 128])
                ob_ref[cur, j, :, tile * tq:(tile + 1) * tq] = of.astype(ob_ref.dtype)
        store_carry(tt0)
        return allfast[0, 0]

    zero = jnp.int32(0)
    q0_copy = pltpu.make_async_copy(q_hbm.at[0], qb_ref.at[0], sem.at[3])
    k0_copy = pltpu.make_async_copy(k_hbm.at[0], kb_ref.at[0], sem.at[4])
    q0_copy.start()
    k0_copy.start()
    prefetch(zero - 1)
    ok = probe()
    q0_copy.wait()
    k0_copy.wait()
    fast0 = full_prep(zero) * ok

    def sync(b):
        v_copy(b).wait()
        q_copy(b + 1).wait()
        k_copy(b + 1).wait()

        @pl.when(b >= 1)
        def _():
            for j in range(HB - 1):
                o_copy(b - 1, j).wait()

        @pl.when(b >= 2)
        def _():
            o_copy(b - 2, HB - 1).wait()

    def body(b, fast):
        sync(b)
        return lax.cond(fast == 1, packed_block, exact_block, b) * ok

    lax.fori_loop(0, NB, body, fast0)
    last = jnp.int32(NB)
    sync(last)
    o_copy(last - 1, HB - 1).start()
    o_copy(last - 1, HB - 1).wait()


@jax.jit
def pallas_standalone__fused_io_aware_attn__prompt_kernel(
    q: jax.Array,
    k: jax.Array,
    v: jax.Array,
):
    B, H, S, D = q.shape
    NB = B * H // HB
    qT, kT, vT = (jnp.swapaxes(x, -1, -2).reshape(NB, HB, D, S) for x in (q, k, v))
    hbm = pl.BlockSpec(memory_space=pl.ANY)
    oT = pl.pallas_call(
        _attn_kernel,
        in_specs=[hbm, hbm, hbm],
        out_specs=hbm,
        out_shape=jax.ShapeDtypeStruct((NB, HB, D, S), q.dtype),
        scratch_shapes=[
            pltpu.VMEM((2, HB, D, S), BF16),
            pltpu.VMEM((4, HB, D, S), BF16),
            pltpu.VMEM((2, HB, D, S), BF16),
            pltpu.VMEM((2, HB, D, S), BF16),
            pltpu.SemaphoreType.DMA((3 + HB,)),
            pltpu.VMEM((2, HB, S // 4, KA), U32),
            pltpu.VMEM((2, HB, S // TQ, D // 2, TQ), U32),
            pltpu.VMEM((2, HB, D // 2, S), U32),
            pltpu.VMEM((2, TK, TQ), BF16),
            pltpu.VMEM((2, 8, TQ), F32),
            pltpu.VMEM((2, HB, 8, 128), F32),
            pltpu.VMEM((2, HB, 2, 8, 128), U32),
            pltpu.VMEM((S, TQ), F32),
            pltpu.VMEM((HB, S // 2, D), U32),
        ],
        compiler_params=pltpu.CompilerParams(
            disable_bounds_checks=True,
            vmem_limit_bytes=64 * 1024 * 1024),
    )(qT, kT, vT)
    return jnp.swapaxes(oT.reshape(B, H, D, S), -1, -2)
```

```python
import functools
import math

import jax
import jax.numpy as jnp
from jax import lax
import jax.experimental.pallas as pl
import jax.experimental.pallas.tpu as pltpu

F32, BF16, U32, I32 = jnp.float32, jnp.bfloat16, jnp.uint32, jnp.int32

HB = 2
TQ = 256
TQE = 512
TK = 128
KA = 96
EPS = 2.0 ** -11
XMAX = 4
MARGIN = 0.97
CPS = 2
LEAD = 3

Q0, QSTEP, K0, KSTEP, V0, VSTEP, FIN = 14, 1, 10, 2, 8, 3, 55
TIE_LAG, V_TIE, V_PROG = 4, 3, 2


def _attn_kernel(q_hbm, k_hbm, v_hbm, o_hbm,
                 qb_ref, kb_ref, vb_ref, ob_ref, sem,
                 kt_ref, w_ref, vh_ref, p0_ref, l0_ref, up_ref, cw_ref,
                 s_ref, kr_ref):
    NB, _, D, S = q_hbm.shape
    tq, tk = TQ, TK
    c = (D ** -0.5) * math.log2(math.e)
    nq = S // tq
    nc = S // tk
    ng = tk // 16
    lo0 = D + 16

    def tile4(z, width=TQ):
        return jnp.concatenate([z] * (width // 128), axis=1)

    def q_copy(b):
        return pltpu.make_async_copy(
            q_hbm.at[jnp.minimum(b, NB - 1)], qb_ref.at[b & 1], sem.at[0])

    def k_copy(b):
        return pltpu.make_async_copy(
            k_hbm.at[jnp.minimum(b, NB - 1)], kb_ref.at[b & 3], sem.at[1])

    def v_copy(b):
        return pltpu.make_async_copy(
            v_hbm.at[jnp.minimum(b, NB - 1)], vb_ref.at[b & 1], sem.at[2])

    def o_copy(b, j):
        return pltpu.make_async_copy(
            ob_ref.at[b & 1, j], o_hbm.at[b, j], sem.at[3 + j])

    def prefetch(b):
        @pl.when(b >= 1)
        def _():
            o_copy(b - 1, HB - 1).start()

        v_copy(b + 1).start()
        q_copy(b + 2).start()
        k_copy(b + 2).start()

    def pack_lhs(ks):
        row = lax.broadcasted_iota(I32, (8, tk), 0)
        lane = lax.broadcasted_iota(I32, (8, KA), 1)
        e0 = jnp.where(row == 0, 1.0, 0.0)
        e01 = jnp.where(row < 2, 1.0, 0.0)
        aug = jnp.concatenate(
            [ks, e0, e0, ks * EPS, e01, jnp.zeros_like(e0)], axis=0).astype(BF16)
        z = pltpu.bitcast(aug.T, U32)
        out = []
        for i in range(ng // 2):
            hi_g, lo_g = ng - 1 - 2 * i, ng - 2 - 2 * i
            out.append(jnp.where(lane < lo0, z[8 * hi_g:8 * hi_g + 8],
                                 z[8 * lo_g:8 * lo_g + 8]))
        return out

    def prep_k(bn, j, ci, run):
        ks = kb_ref[bn & 3, j, :, pl.ds(ci * tk, tk)].astype(F32) * c
        for i, zz in enumerate(pack_lhs(ks)):
            kt_ref[bn & 1, j, pl.ds(ci * 32 + 8 * i, 8), :] = zz
        n2 = jnp.sum(ks * ks, axis=0, keepdims=True)
        return n2 if run is None else jnp.maximum(run, n2)

    def prep_q(bn, j, i, run):
        qb = qb_ref[bn & 1, j, :, i * 128:(i + 1) * 128]
        w_ref[bn & 1, j, :, i * 128:(i + 1) * 128] = pltpu.bitcast(qb, U32)
        x = qb.astype(F32)
        n2 = jnp.sum(x * x, axis=0, keepdims=True)
        return n2 if run is None else jnp.maximum(run, n2)

    def const_rows(p2):
        row = lax.broadcasted_iota(I32, (8, 128), 0)
        a0 = jnp.where(row == 0, 1.5 * 2.0 ** 12, 0.0) * p2
        b0 = jnp.where(row == 0, -1.5, jnp.where(row == 1, -(2.0 ** -12), 0.0)) * p2
        wa = jnp.concatenate([a0, -a0], axis=0).astype(BF16)
        wb = jnp.concatenate([b0, jnp.zeros_like(b0)], axis=0).astype(BF16)
        return pltpu.bitcast(wa, U32), pltpu.bitcast(wb, U32)

    def prep_scale(bn, j, rq, rk):
        mq = jnp.max(rq, axis=1, keepdims=True) + 2.0 ** -100
        mk = jnp.max(rk, axis=1, keepdims=True) + 2.0 ** -100
        b2 = jnp.broadcast_to(mq * mk, (8, 128))
        p2 = jnp.full((8, 128), 2.0 ** XMAX, F32)
        up = jnp.full((8, 128), 2.0 ** (2 ** XMAX), F32)
        for x in reversed(range(XMAX)):
            ok = b2 <= (MARGIN * 2.0 ** (x - 1)) ** 2
            p2 = jnp.where(ok, 2.0 ** x, p2)
            up = jnp.where(ok, 2.0 ** (2 ** x), up)
        fast = jnp.where(b2 <= (MARGIN * 2.0 ** (XMAX - 1)) ** 2, 1, 0).astype(I32)
        consts = const_rows(p2)
        up_ref[bn & 1, j] = up
        cw_ref[bn & 1, j, 0] = consts[0]
        cw_ref[bn & 1, j, 1] = consts[1]
        return consts, fast

    def packed_dot(kc, wq, consts):
        w = jnp.concatenate([wq, tile4(consts[0]), wq, tile4(consts[1])], axis=0)
        return jnp.dot(pltpu.bitcast(kc, BF16), pltpu.bitcast(w, BF16),
                       preferred_element_type=F32)

    def qk(slot, j, tile, ci, consts):
        return packed_dot(kt_ref[slot, j, pl.ds(ci * 32 * CPS, 32 * CPS), :],
                          w_ref[slot, j, :, tile * tq:(tile + 1) * tq], consts)

    def decode(tt):
        hi = pltpu.bitcast(pltpu.bitcast(tt, U32) & jnp.uint32(0xFFFFF000), F32)
        return hi, (tt - hi) * (1.0 / EPS)

    def exp_chunk(tt, lh, ll):
        hi, lo = decode(tt)
        ph, plo = jnp.exp2(hi), jnp.exp2(lo)
        grp = [None] * (ng * CPS)
        for cc in range(CPS):
            for i in range(ng // 2):
                r0 = 64 * cc + 16 * i
                a = ph[r0:r0 + 8] + ph[r0 + 8:r0 + 16]
                b = plo[r0:r0 + 8] + plo[r0 + 8:r0 + 16]
                lh = a if lh is None else lh + a
                ll = b if ll is None else ll + b
                grp[cc * ng + ng - 1 - 2 * i] = ph[r0:r0 + 16]
                grp[cc * ng + ng - 2 - 2 * i] = plo[r0:r0 + 16]
        return jnp.concatenate(grp, axis=0).astype(BF16), lh, ll

    def store_carry(tt0):
        lh = ll = None
        for e in range(LEAD):
            p, lh, ll = exp_chunk(tt0[e], lh, ll)
            p0_ref[e] = p
        l0_ref[0] = lh
        l0_ref[1] = ll

    def full_prep(bn):
        allfast = None
        for j in range(HB):
            rq = rk = None
            for i in range(nc):
                rq = prep_q(bn, j, i, rq)
            for ci in range(nc):
                rk = prep_k(bn, j, ci, rk)
            consts, fast = prep_scale(bn, j, rq, rk)
            if j == 0:
                store_carry([qk(bn & 1, 0, 0, e, consts) for e in range(LEAD)])
            allfast = fast if allfast is None else allfast * fast
        return allfast[0, 0]

    def probe():
        r = lax.broadcasted_iota(I32, (D, tk), 0)
        cc = lax.broadcasted_iota(I32, (D, tk), 1)
        ks = (((r * 37 + cc * 11) & 127) - 63).astype(F32) * (2.0 ** -9)
        r = lax.broadcasted_iota(I32, (D, tq), 0)
        cc = lax.broadcasted_iota(I32, (D, tq), 1)
        kc = jnp.concatenate(pack_lhs(ks) * CPS, axis=0)
        consts = const_rows(jnp.ones((8, 128), F32))
        err = None
        for rep in range(2):
            qs = (((r * 29 + cc * (13 + 4 * rep)) & 127) - 63).astype(F32) * (2.0 ** -10)
            qs = qs.astype(BF16)
            hi, lo = decode(packed_dot(kc, pltpu.bitcast(qs, U32), consts))
            ex = lax.dot_general(ks.astype(BF16), qs, (((0,), (0,)), ((), ())),
                                 preferred_element_type=F32)
            for i in range(CPS * ng // 2):
                hi_g, lo_g = ng - 1 - 2 * (i % 4), ng - 2 - 2 * (i % 4)
                e1 = jnp.abs(hi[16 * i:16 * i + 16] + 1.5 - ex[16 * hi_g:16 * hi_g + 16])
                e2 = jnp.abs(lo[16 * i:16 * i + 16] + 0.5 - ex[16 * lo_g:16 * lo_g + 16])
                e = jnp.maximum(e1, e2)
                err = e if err is None else jnp.maximum(err, e)
        bad = jnp.where(err <= 2.0 ** -11, 0.0, 1.0)
        return jnp.where(jnp.max(bad) == 0.0, 1, 0).astype(I32)

    def exact_block(b):
        prefetch(b)
        cur = b & 1
        tq, nq = TQE, S // TQE
        n_tiles = HB * nq
        always = tile4(up_ref[cur, 0], tq) > 0.0
        for j in range(HB):
            for ci in range(nc):
                kr_ref[j, pl.ds(ci * 64, 64), :] = pltpu.bitcast(
                    kb_ref[b & 3, j, :, pl.ds(ci * tk, tk)].T, U32)

        def stage(it_qk, it_pv, m):
            if it_qk is not None:
                jq = it_qk // nq
                qoff = pl.multiple_of((it_qk % nq) * tq, tq)
                wq = pltpu.bitcast(w_ref[cur, jq, :, pl.ds(qoff, tq)], BF16)
            if it_pv is not None:
                jv = it_pv // nq
            m8 = l8 = acc = prev = None
            for ci in range(nc):
                if it_pv is not None:
                    s_cur = s_ref[pl.ds(ci * tk, tk), :]
                cm = None
                if it_qk is not None:
                    kc = pltpu.bitcast(kr_ref[jq, pl.ds(ci * 64, 64), :], BF16)
                    s = jnp.dot(kc, wq, preferred_element_type=F32)
                    s_ref[pl.ds(ci * tk, tk), :] = s
                    cm = [jnp.maximum(s[16 * r:16 * r + 8], s[16 * r + 8:16 * r + 16])
                          for r in range(ng)]
                    for a in cm:
                        m8 = a if m8 is None else jnp.maximum(m8, a)
                if it_pv is not None:
                    ps = [None] * ng
                    for i, r in enumerate(reversed(range(ng))):
                        if i % 2 == 0:
                            mg = m if prev is None else jnp.where(always, m, prev[i])
                        pa = jnp.exp2((s_cur[16 * r:16 * r + 8] - mg) * c)
                        pb = jnp.exp2((s_cur[16 * r + 8:16 * r + 16] - mg) * c)
                        l8 = pa + pb if l8 is None else l8 + (pa + pb)
                        ps[r] = jnp.concatenate([pa, pb], axis=0)
                    p = jnp.concatenate(ps, axis=0).astype(BF16)
                    pv = jnp.dot(vb_ref[cur, jv, :, pl.ds(ci * tk, tk)], p,
                                 preferred_element_type=F32)
                    acc = pv if acc is None else pv + acc
                prev = cm
            if it_pv is not None:
                l = jnp.sum(l8, axis=0, keepdims=True)
                off = pl.multiple_of((it_pv % nq) * tq, tq)
                ob_ref[cur, jv, :, pl.ds(off, tq)] = (acc * (1.0 / l)).astype(ob_ref.dtype)
            if it_qk is None:
                return None
            return jnp.broadcast_to(jnp.max(m8, axis=0, keepdims=True), (8, tq))

        m = stage(0, None, None)
        nfast = full_prep(b + 1)
        m = lax.fori_loop(0, n_tiles - 1, lambda i, mm: stage(i + 1, i, mm), m)
        for j in range(HB - 1):
            o_copy(b, j).start()
        stage(None, n_tiles - 1, m)
        return nfast

    def packed_block(b):
        cur = b & 1
        bn = b + 1
        consts = [(cw_ref[cur, j, 0], cw_ref[cur, j, 1]) for j in range(HB)]
        ups = [up_ref[cur, j] for j in range(HB)]
        lane = lax.broadcasted_iota(I32, (8, tk), 1)
        odd = (lane // 16) % 2 == 1

        always = ups[0] > 0.0
        ties = {}

        def tie(e, val):
            if val.dtype != U32:
                val = pltpu.bitcast(jnp.broadcast_to(val, (8, 128)), U32)
            ties.setdefault(e, []).append(val)

        def prep_v(j, ci, e_tie):
            upv = jnp.where(odd, ups[j], 1.0)
            vf = vb_ref[cur, j, :, pl.ds(ci * tk, tk)].astype(F32)
            vf = (vf.reshape(D // 8, 8, tk) * upv[None]).reshape(D, tk)
            vhu = pltpu.bitcast(vf.astype(BF16), U32)
            vh_ref[cur, j, :, pl.ds(ci * tk, tk)] = vhu
            if e_tie is not None:
                tie(e_tie, vhu[0:8])
                tie(e_tie, vhu[8:16])

        ns = nc // CPS
        per_head = nq * ns
        n_steps = HB * per_head
        tts, tt0, runs = {}, [], []
        lh = ll = acc = rq = rk = allfast = nconsts0 = None
        for e in range(n_steps):
            j, el = divmod(e, per_head)
            tile, ci = divmod(el, ns)
            if e + LEAD < n_steps:
                j1, el1 = divmod(e + LEAD, per_head)
                t1, c1 = divmod(el1, ns)
                cb = consts[j1][1]
                vals = ties.pop(e + 2, [])
                if vals:
                    cb = jnp.where(always, cb, functools.reduce(jnp.bitwise_or, vals))
                tts[e + LEAD] = qk(cur, j1, t1, c1, (consts[j1][0], cb))
            else:
                tt0.append(qk(bn & 1, 0, 0, e + LEAD - n_steps, nconsts0))
            if e == 0:
                prefetch(b)
                for cv in range(nc):
                    et = V_TIE + cv // V_PROG
                    prep_v(0, cv, et if et < cv // CPS + 2 else None)
            if j >= 1 and el == 8:
                o_copy(b, j - 1).start()
            jp = (j + 1) % HB
            if el == 0:
                rq = rk = None
            if (el - Q0) % QSTEP == 0 and 0 <= (el - Q0) // QSTEP < nc:
                rq = prep_q(bn, jp, (el - Q0) // QSTEP, rq)
                tie(e + TIE_LAG, rq)
            if (el - K0) % KSTEP == 0 and 0 <= (el - K0) // KSTEP < nc:
                rk = prep_k(bn, jp, (el - K0) // KSTEP, rk)
                tie(e + TIE_LAG, rk)
            if j + 1 < HB and (el - V0) % VSTEP == 0 and 0 <= (el - V0) // VSTEP < nc:
                prep_v(j + 1, (el - V0) // VSTEP, e + TIE_LAG)
            if el == FIN:
                runs.append((jp, rq, rk))
                if j == HB - 1:
                    for jn, rqn, rkn in runs:
                        nconsts, fast = prep_scale(bn, jn, rqn, rkn)
                        tie(e + TIE_LAG, nconsts[0])
                        tie(e + TIE_LAG, nconsts[1])
                        if jn == 0:
                            nconsts0 = nconsts
                        allfast = fast if allfast is None else allfast * fast
            if ci == 0:
                lh = ll = None
            if e == 0:
                lh, ll = l0_ref[0], l0_ref[1]
            if e < LEAD:
                p = p0_ref[e]
            else:
                p, lh, ll = exp_chunk(tts.pop(e), lh, ll)
            vh = pltpu.bitcast(vh_ref[cur, j, :, pl.ds(ci * tk * CPS, tk * CPS)], BF16)
            pv = jnp.dot(vh, p, preferred_element_type=F32)
            acc = pv if ci == 0 else pv + acc
            if ci == ns - 1:
                l = jnp.sum(lh * tile4(ups[j]) + ll, axis=0, keepdims=True)
                r0 = pl.reciprocal(l, approx=True)
                rinv = r0 * (2.0 - l * r0)
                ob_ref[cur, j, :, tile * tq:(tile + 1) * tq] = (acc * rinv).astype(ob_ref.dtype)
        store_carry(tt0)
        return allfast[0, 0]

    zero = jnp.int32(0)
    q0_copy = pltpu.make_async_copy(q_hbm.at[0], qb_ref.at[0], sem.at[3])
    k0_copy = pltpu.make_async_copy(k_hbm.at[0], kb_ref.at[0], sem.at[4])
    q0_copy.start()
    k0_copy.start()
    prefetch(zero - 1)
    ok = probe()
    q0_copy.wait()
    k0_copy.wait()
    fast0 = full_prep(zero) * ok

    def sync(b):
        v_copy(b).wait()
        q_copy(b + 1).wait()
        k_copy(b + 1).wait()

        @pl.when(b >= 1)
        def _():
            for j in range(HB - 1):
                o_copy(b - 1, j).wait()

        @pl.when(b >= 2)
        def _():
            o_copy(b - 2, HB - 1).wait()

    def body(b, fast):
        sync(b)
        return lax.cond(fast == 1, packed_block, exact_block, b) * ok

    lax.fori_loop(0, NB, body, fast0)
    last = jnp.int32(NB)
    sync(last)
    o_copy(last - 1, HB - 1).start()
    o_copy(last - 1, HB - 1).wait()


@jax.jit
def pallas_standalone__fused_io_aware_attn__prompt_kernel(
    q: jax.Array,
    k: jax.Array,
    v: jax.Array,
):
    B, H, S, D = q.shape
    NB = B * H // HB
    qT, kT, vT = (jnp.swapaxes(x, -1, -2).reshape(NB, HB, D, S) for x in (q, k, v))
    hbm = pl.BlockSpec(memory_space=pl.ANY)
    oT = pl.pallas_call(
        _attn_kernel,
        in_specs=[hbm, hbm, hbm],
        out_specs=hbm,
        out_shape=jax.ShapeDtypeStruct((NB, HB, D, S), q.dtype),
        scratch_shapes=[
            pltpu.VMEM((2, HB, D, S), BF16),
            pltpu.VMEM((4, HB, D, S), BF16),
            pltpu.VMEM((2, HB, D, S), BF16),
            pltpu.VMEM((2, HB, D, S), BF16),
            pltpu.SemaphoreType.DMA((3 + HB,)),
            pltpu.VMEM((2, HB, S // 4, KA), U32),
            pltpu.VMEM((2, HB, D // 2, S), U32),
            pltpu.VMEM((2, HB, D // 2, S), U32),
            pltpu.VMEM((LEAD, TK * CPS, TQ), BF16),
            pltpu.VMEM((2, 8, TQ), F32),
            pltpu.VMEM((2, HB, 8, 128), F32),
            pltpu.VMEM((2, HB, 2, 8, 128), U32),
            pltpu.VMEM((S, TQE), F32),
            pltpu.VMEM((HB, S // 2, D), U32),
        ],
        compiler_params=pltpu.CompilerParams(
            disable_bounds_checks=True,
            vmem_limit_bytes=64 * 1024 * 1024),
    )(qT, kT, vT)
    return jnp.swapaxes(oT.reshape(B, H, D, S), -1, -2)
```

```python
import functools
import math

import jax
import jax.numpy as jnp
from jax import lax
import jax.experimental.pallas as pl
import jax.experimental.pallas.tpu as pltpu

F32, BF16, U32, I32 = jnp.float32, jnp.bfloat16, jnp.uint32, jnp.int32

HB = 2
TK = 128
TQE = 512
TQ = 256
CPS = 2
LEAD = 3
KA = 96
EPS = 2.0 ** -11
XMAX = 4
MARGIN = 0.97

Q0, QSTEP, K0, KSTEP, V0, VSTEP, FIN, TIE_LAG = 14, 1, 10, 2, 8, 3, 55, 4


def _attn_kernel(q_hbm, k_hbm, v_hbm, o_hbm,
                 qb_ref, kb_ref, vb_ref, ob_ref, sem,
                 kt_ref, w_ref, vh_ref, p0_ref, l0_ref, up_ref, cw_ref,
                 s_ref, kr_ref):
    NB, _, D, S = q_hbm.shape
    tq, tk = TQ, TK
    c = (D ** -0.5) * math.log2(math.e)
    nq = S // tq
    nc = S // tk
    ng = tk // 16
    lo0 = D + 16

    def widen(z, width=TQ):
        return jnp.concatenate([z] * (width // 128), axis=1)

    def q_copy(b):
        return pltpu.make_async_copy(
            q_hbm.at[jnp.minimum(b, NB - 1)], qb_ref.at[b & 1], sem.at[0])

    def k_copy(b):
        return pltpu.make_async_copy(
            k_hbm.at[jnp.minimum(b, NB - 1)], kb_ref.at[b & 3], sem.at[1])

    def v_copy(b):
        return pltpu.make_async_copy(
            v_hbm.at[jnp.minimum(b, NB - 1)], vb_ref.at[b & 1], sem.at[2])

    def o_copy(b, j):
        return pltpu.make_async_copy(
            ob_ref.at[b & 1, j], o_hbm.at[b, j], sem.at[3 + j])

    def prefetch(b):
        v_copy(b + 1).start()
        q_copy(b + 2).start()
        k_copy(b + 2).start()

    def start_copies(b):
        @pl.when(b >= 1)
        def _():
            o_copy(b - 1, HB - 1).start()

        prefetch(b)

    def pack_lhs(ks):
        row = lax.broadcasted_iota(I32, (8, tk), 0)
        lane = lax.broadcasted_iota(I32, (8, KA), 1)
        e0 = jnp.where(row == 0, 1.0, 0.0)
        e01 = jnp.where(row < 2, 1.0, 0.0)
        aug = jnp.concatenate(
            [ks, e0, e0, ks * EPS, e01, jnp.zeros_like(e0)], axis=0).astype(BF16)
        z = pltpu.bitcast(aug.T, U32)
        out = []
        for i in range(ng // 2):
            hi_g, lo_g = ng - 1 - 2 * i, ng - 2 - 2 * i
            out.append(jnp.where(lane < lo0, z[8 * hi_g:8 * hi_g + 8],
                                 z[8 * lo_g:8 * lo_g + 8]))
        return out

    def prep_k(bn, j, ci, run):
        ks = kb_ref[bn & 3, j, :, pl.ds(ci * tk, tk)].astype(F32) * c
        for i, zz in enumerate(pack_lhs(ks)):
            kt_ref[bn & 1, j, pl.ds(ci * 32 + 8 * i, 8), :] = zz
        n2 = jnp.sum(ks * ks, axis=0, keepdims=True)
        return n2 if run is None else jnp.maximum(run, n2)

    def prep_q(bn, j, i, run):
        qb = qb_ref[bn & 1, j, :, i * 128:(i + 1) * 128]
        w_ref[bn & 1, j, :, i * 128:(i + 1) * 128] = pltpu.bitcast(qb, U32)
        x = qb.astype(F32)
        n2 = jnp.sum(x * x, axis=0, keepdims=True)
        return n2 if run is None else jnp.maximum(run, n2)

    def const_rows(p2):
        row = lax.broadcasted_iota(I32, (8, 128), 0)
        a0 = jnp.where(row == 0, 1.5 * 2.0 ** 12, 0.0) * p2
        b0 = jnp.where(row == 0, -1.5, jnp.where(row == 1, -(2.0 ** -12), 0.0)) * p2
        wa = jnp.concatenate([a0, -a0], axis=0).astype(BF16)
        wb = jnp.concatenate([b0, jnp.zeros_like(b0)], axis=0).astype(BF16)
        return pltpu.bitcast(wa, U32), pltpu.bitcast(wb, U32)

    def prep_scale(bn, j, rq, rk):
        mq = jnp.max(rq, axis=1, keepdims=True) + 2.0 ** -100
        mk = jnp.max(rk, axis=1, keepdims=True) + 2.0 ** -100
        b2 = jnp.broadcast_to(mq * mk, (8, 128))
        p2 = jnp.full((8, 128), 2.0 ** XMAX, F32)
        up = jnp.full((8, 128), 2.0 ** (2 ** XMAX), F32)
        for x in reversed(range(XMAX)):
            ok = b2 <= (MARGIN * 2.0 ** (x - 1)) ** 2
            p2 = jnp.where(ok, 2.0 ** x, p2)
            up = jnp.where(ok, 2.0 ** (2 ** x), up)
        fast = jnp.where(b2 <= (MARGIN * 2.0 ** (XMAX - 1)) ** 2, 1, 0).astype(I32)
        consts = const_rows(p2)
        up_ref[bn & 1, j] = up
        cw_ref[bn & 1, j, 0] = consts[0]
        cw_ref[bn & 1, j, 1] = consts[1]
        return consts, fast

    def packed_dot(kc, wq, consts):
        w = jnp.concatenate([wq, widen(consts[0]), wq, widen(consts[1])], axis=0)
        return jnp.dot(pltpu.bitcast(kc, BF16), pltpu.bitcast(w, BF16),
                       preferred_element_type=F32)

    def qk(slot, j, tile, ci, consts):
        return packed_dot(kt_ref[slot, j, pl.ds(ci * 32 * CPS, 32 * CPS), :],
                          w_ref[slot, j, :, tile * tq:(tile + 1) * tq], consts)

    def decode(tt):
        hi = pltpu.bitcast(pltpu.bitcast(tt, U32) & jnp.uint32(0xFFFFF000), F32)
        return hi, (tt - hi) * (1.0 / EPS)

    def exp_chunk(tt, lh, ll):
        hi, lo = decode(tt)
        ph, plo = jnp.exp2(hi), jnp.exp2(lo)
        grp = [None] * (ng * CPS)
        for cc in range(CPS):
            for i in range(ng // 2):
                r0 = 64 * cc + 16 * i
                a = ph[r0:r0 + 8] + ph[r0 + 8:r0 + 16]
                b = plo[r0:r0 + 8] + plo[r0 + 8:r0 + 16]
                lh = a if lh is None else lh + a
                ll = b if ll is None else ll + b
                grp[cc * ng + ng - 1 - 2 * i] = ph[r0:r0 + 16]
                grp[cc * ng + ng - 2 - 2 * i] = plo[r0:r0 + 16]
        return jnp.concatenate(grp, axis=0).astype(BF16), lh, ll

    def store_carry(tt0):
        lh = ll = None
        for e in range(LEAD):
            p, lh, ll = exp_chunk(tt0[e], lh, ll)
            p0_ref[e] = p
        l0_ref[0] = lh
        l0_ref[1] = ll

    def full_prep(bn):
        allfast = None
        for j in range(HB):
            rq = rk = None
            for i in range(nc):
                rq = prep_q(bn, j, i, rq)
            for ci in range(nc):
                rk = prep_k(bn, j, ci, rk)
            consts, fast = prep_scale(bn, j, rq, rk)
            if j == 0:
                store_carry([qk(bn & 1, 0, 0, e, consts) for e in range(LEAD)])
            allfast = fast if allfast is None else allfast * fast
        return allfast[0, 0]

    def probe():
        r = lax.broadcasted_iota(I32, (D, tk), 0)
        cc = lax.broadcasted_iota(I32, (D, tk), 1)
        ks = (((r * 37 + cc * 11) & 127) - 63).astype(F32) * (2.0 ** -9)
        r = lax.broadcasted_iota(I32, (D, tq), 0)
        cc = lax.broadcasted_iota(I32, (D, tq), 1)
        kc = jnp.concatenate(pack_lhs(ks) * CPS, axis=0)
        consts = const_rows(jnp.ones((8, 128), F32))
        err = None
        for rep in range(2):
            qs = (((r * 29 + cc * (13 + 4 * rep)) & 127) - 63).astype(F32) * (2.0 ** -10)
            qs = qs.astype(BF16)
            hi, lo = decode(packed_dot(kc, pltpu.bitcast(qs, U32), consts))
            ex = lax.dot_general(ks.astype(BF16), qs, (((0,), (0,)), ((), ())),
                                 preferred_element_type=F32)
            for i in range(CPS * ng // 2):
                hi_g, lo_g = ng - 1 - 2 * (i % 4), ng - 2 - 2 * (i % 4)
                e1 = jnp.abs(hi[16 * i:16 * i + 16] + 1.5 - ex[16 * hi_g:16 * hi_g + 16])
                e2 = jnp.abs(lo[16 * i:16 * i + 16] + 0.5 - ex[16 * lo_g:16 * lo_g + 16])
                e = jnp.maximum(e1, e2)
                err = e if err is None else jnp.maximum(err, e)
        bad = jnp.where(err <= 2.0 ** -11, 0.0, 1.0)
        return jnp.where(jnp.max(bad) == 0.0, 1, 0).astype(I32)

    def exact_block(b):
        start_copies(b)
        cur = b & 1
        tq, nq = TQE, S // TQE
        n_tiles = HB * nq
        always = widen(up_ref[cur, 0], tq) > 0.0
        for j in range(HB):
            for ci in range(nc):
                kr_ref[j, pl.ds(ci * 64, 64), :] = pltpu.bitcast(
                    kb_ref[b & 3, j, :, pl.ds(ci * tk, tk)].T, U32)

        def stage(it_qk, it_pv, m):
            if it_qk is not None:
                jq = it_qk // nq
                qoff = pl.multiple_of((it_qk % nq) * tq, tq)
                wq = pltpu.bitcast(w_ref[cur, jq, :, pl.ds(qoff, tq)], BF16)
            if it_pv is not None:
                jv = it_pv // nq
            m8 = l8 = acc = prev = None
            for ci in range(nc):
                if it_pv is not None:
                    s_cur = s_ref[pl.ds(ci * tk, tk), :]
                cm = None
                if it_qk is not None:
                    kc = pltpu.bitcast(kr_ref[jq, pl.ds(ci * 64, 64), :], BF16)
                    s = jnp.dot(kc, wq, preferred_element_type=F32)
                    s_ref[pl.ds(ci * tk, tk), :] = s
                    cm = [jnp.maximum(s[16 * r:16 * r + 8], s[16 * r + 8:16 * r + 16])
                          for r in range(ng)]
                    for a in cm:
                        m8 = a if m8 is None else jnp.maximum(m8, a)
                if it_pv is not None:
                    ps = [None] * ng
                    for i, r in enumerate(reversed(range(ng))):
                        if i % 2 == 0:
                            mg = m if prev is None else jnp.where(always, m, prev[i])
                        pa = jnp.exp2((s_cur[16 * r:16 * r + 8] - mg) * c)
                        pb = jnp.exp2((s_cur[16 * r + 8:16 * r + 16] - mg) * c)
                        l8 = pa + pb if l8 is None else l8 + (pa + pb)
                        ps[r] = jnp.concatenate([pa, pb], axis=0)
                    p = jnp.concatenate(ps, axis=0).astype(BF16)
                    pv = jnp.dot(vb_ref[cur, jv, :, pl.ds(ci * tk, tk)], p,
                                 preferred_element_type=F32)
                    acc = pv if acc is None else pv + acc
                prev = cm
            if it_pv is not None:
                l = jnp.sum(l8, axis=0, keepdims=True)
                off = pl.multiple_of((it_pv % nq) * tq, tq)
                ob_ref[cur, jv, :, pl.ds(off, tq)] = (acc * (1.0 / l)).astype(ob_ref.dtype)
            if it_qk is None:
                return None
            return jnp.broadcast_to(jnp.max(m8, axis=0, keepdims=True), (8, tq))

        m = stage(0, None, None)
        nfast = full_prep(b + 1)
        m = lax.fori_loop(0, n_tiles - 1, lambda i, mm: stage(i + 1, i, mm), m)
        for j in range(HB - 1):
            o_copy(b, j).start()
        stage(None, n_tiles - 1, m)
        return nfast

    def packed_block(b):
        cur = b & 1
        bn = b + 1
        consts = [(cw_ref[cur, j, 0], cw_ref[cur, j, 1]) for j in range(HB)]
        ups = [up_ref[cur, j] for j in range(HB)]
        lane = lax.broadcasted_iota(I32, (8, tk), 1)
        odd = (lane // 16) % 2 == 1

        always = ups[0] > 0.0
        ties = {}

        def tie(e, val):
            if val.dtype != U32:
                val = pltpu.bitcast(jnp.broadcast_to(val, (8, 128)), U32)
            ties.setdefault(e, []).append(val)

        def prep_v(j, ci, e_tie):
            upv = jnp.where(odd, ups[j], 1.0)
            vf = vb_ref[cur, j, :, pl.ds(ci * tk, tk)].astype(F32)
            vf = (vf.reshape(D // 8, 8, tk) * upv[None]).reshape(D, tk)
            vhu = pltpu.bitcast(vf.astype(BF16), U32)
            vh_ref[cur, j, :, pl.ds(ci * tk, tk)] = vhu
            if e_tie is not None:
                tie(e_tie, vhu[0:8])
                tie(e_tie, vhu[8:16])

        ns = nc // CPS
        per_head = nq * ns
        n_steps = HB * per_head
        tts, tt0, runs = {}, [], []
        lh = ll = acc = rq = rk = allfast = nconsts0 = None
        for e in range(n_steps):
            j, el = divmod(e, per_head)
            tile, ci = divmod(el, ns)
            if e + LEAD < n_steps:
                j1, el1 = divmod(e + LEAD, per_head)
                t1, c1 = divmod(el1, ns)
                cb = consts[j1][1]
                vals = ties.pop(e + 2, [])
                if vals:
                    cb = jnp.where(always, cb, functools.reduce(jnp.bitwise_or, vals))
                tts[e + LEAD] = qk(cur, j1, t1, c1, (consts[j1][0], cb))
            else:
                tt0.append(qk(bn & 1, 0, 0, e + LEAD - n_steps, nconsts0))
            if e == 0:
                start_copies(b)
                for cv in range(nc):
                    prep_v(0, cv, None)
            if j >= 1 and el == 8:
                o_copy(b, j - 1).start()
            jp = (j + 1) % HB
            if el == 0:
                rq = rk = None
            if (el - Q0) % QSTEP == 0 and 0 <= (el - Q0) // QSTEP < nc:
                rq = prep_q(bn, jp, (el - Q0) // QSTEP, rq)
                tie(e + TIE_LAG, rq)
            if (el - K0) % KSTEP == 0 and 0 <= (el - K0) // KSTEP < nc:
                rk = prep_k(bn, jp, (el - K0) // KSTEP, rk)
                tie(e + TIE_LAG, rk)
            if j + 1 < HB and (el - V0) % VSTEP == 0 and 0 <= (el - V0) // VSTEP < nc:
                prep_v(j + 1, (el - V0) // VSTEP, e + TIE_LAG)
            if el == FIN:
                runs.append((jp, rq, rk))
                if j == HB - 1:
                    for jn, rqn, rkn in runs:
                        nconsts, fast = prep_scale(bn, jn, rqn, rkn)
                        tie(e + TIE_LAG, nconsts[0])
                        tie(e + TIE_LAG, nconsts[1])
                        if jn == 0:
                            nconsts0 = nconsts
                        allfast = fast if allfast is None else allfast * fast
            if ci == 0:
                lh = ll = None
            if e == 0:
                lh, ll = l0_ref[0], l0_ref[1]
            if e < LEAD:
                p = p0_ref[e]
            else:
                p, lh, ll = exp_chunk(tts.pop(e), lh, ll)
            vh = pltpu.bitcast(vh_ref[cur, j, :, pl.ds(ci * tk * CPS, tk * CPS)], BF16)
            pv = jnp.dot(vh, p, preferred_element_type=F32)
            acc = pv if ci == 0 else pv + acc
            if ci == ns - 1:
                l = jnp.sum(lh * widen(ups[j]) + ll, axis=0, keepdims=True)
                r0 = pl.reciprocal(l, approx=True)
                rinv = r0 * (2.0 - l * r0)
                ob_ref[cur, j, :, tile * tq:(tile + 1) * tq] = (acc * rinv).astype(ob_ref.dtype)
        store_carry(tt0)
        return allfast[0, 0]

    zero = jnp.int32(0)
    q0_copy = pltpu.make_async_copy(q_hbm.at[0], qb_ref.at[0], sem.at[3])
    k0_copy = pltpu.make_async_copy(k_hbm.at[0], kb_ref.at[0], sem.at[4])
    q0_copy.start()
    k0_copy.start()
    prefetch(zero - 1)
    ok = probe()
    q0_copy.wait()
    k0_copy.wait()
    fast0 = full_prep(zero) * ok

    def sync(b):
        v_copy(b).wait()
        q_copy(b + 1).wait()
        k_copy(b + 1).wait()

        @pl.when(b >= 1)
        def _():
            for j in range(HB - 1):
                o_copy(b - 1, j).wait()

        @pl.when(b >= 2)
        def _():
            o_copy(b - 2, HB - 1).wait()

    def body(b, fast):
        sync(b)
        return lax.cond(fast == 1, packed_block, exact_block, b) * ok

    lax.fori_loop(0, NB, body, fast0)
    last = jnp.int32(NB)
    sync(last)
    o_copy(last - 1, HB - 1).start()
    o_copy(last - 1, HB - 1).wait()


@jax.jit
def pallas_standalone__fused_io_aware_attn__prompt_kernel(
    q: jax.Array,
    k: jax.Array,
    v: jax.Array,
):
    B, H, S, D = q.shape
    NB = B * H // HB
    qT, kT, vT = (jnp.swapaxes(x, -1, -2).reshape(NB, HB, D, S) for x in (q, k, v))
    hbm = pl.BlockSpec(memory_space=pl.ANY)
    oT = pl.pallas_call(
        _attn_kernel,
        in_specs=[hbm, hbm, hbm],
        out_specs=hbm,
        out_shape=jax.ShapeDtypeStruct((NB, HB, D, S), q.dtype),
        scratch_shapes=[
            pltpu.VMEM((2, HB, D, S), BF16),
            pltpu.VMEM((4, HB, D, S), BF16),
            pltpu.VMEM((2, HB, D, S), BF16),
            pltpu.VMEM((2, HB, D, S), BF16),
            pltpu.SemaphoreType.DMA((3 + HB,)),
            pltpu.VMEM((2, HB, S // 4, KA), U32),
            pltpu.VMEM((2, HB, D // 2, S), U32),
            pltpu.VMEM((2, HB, D // 2, S), U32),
            pltpu.VMEM((LEAD, TK * CPS, TQ), BF16),
            pltpu.VMEM((2, 8, TQ), F32),
            pltpu.VMEM((2, HB, 8, 128), F32),
            pltpu.VMEM((2, HB, 2, 8, 128), U32),
            pltpu.VMEM((S, TQE), F32),
            pltpu.VMEM((HB, S // 2, D), U32),
        ],
        compiler_params=pltpu.CompilerParams(
            disable_bounds_checks=True,
            vmem_limit_bytes=64 * 1024 * 1024),
    )(qT, kT, vT)
    return jnp.swapaxes(oT.reshape(B, H, D, S), -1, -2)
```

```python
import functools
import math

import jax
import jax.numpy as jnp
from jax import lax
import jax.experimental.pallas as pl
import jax.experimental.pallas.tpu as pltpu

F32, BF16, U32, I32 = jnp.float32, jnp.bfloat16, jnp.uint32, jnp.int32

HB = 2
TK = 128
TQE = 512
TQ = 256
CPS = 2
LEAD = 3
KA = 96
EPS = 2.0 ** -11
XMAX = 4
MARGIN = 0.97

Q0, QSTEP, K0, KSTEP, V0, VSTEP, FIN, TIE_LAG, Z_AT = 14, 1, 20, 2, 11, 3, 56, 3, 58


def _attn_kernel(q_hbm, k_hbm, v_hbm, o_hbm,
                 qb_ref, kb_ref, vb_ref, ob_ref, sem,
                 w_ref, vh_ref, p0_ref, l0_ref, up_ref, cw_ref,
                 s_ref, kr_ref, *kt_refs):
    NB, _, D, S = q_hbm.shape
    tq, tk = TQ, TK
    c = (D ** -0.5) * math.log2(math.e)
    nq = S // tq
    nc = S // tk
    ng = tk // 16
    lo0 = D + 16
    assert KA == 2 * lo0 and HB >= 2 and NB >= 2
    assert max(Q0 + (nc - 1) * QSTEP, K0 + (nc - 1) * KSTEP) < FIN < nq * nc // CPS - LEAD
    assert V0 + (nc - 1) * VSTEP < nq * nc // CPS

    def widen(z, width=TQ):
        return jnp.concatenate([z] * (width // 128), axis=1)

    def q_copy(b):
        return pltpu.make_async_copy(
            q_hbm.at[jnp.minimum(b, NB - 1)], qb_ref.at[b & 1], sem.at[0])

    def k_copy(b):
        return pltpu.make_async_copy(
            k_hbm.at[jnp.minimum(b, NB - 1)], kb_ref.at[b & 3], sem.at[1])

    def v_copy(b):
        return pltpu.make_async_copy(
            v_hbm.at[jnp.minimum(b, NB - 1)], vb_ref.at[b & 1], sem.at[2])

    def o_copy(b, j):
        return pltpu.make_async_copy(
            ob_ref.at[b & 1, j], o_hbm.at[b, j], sem.at[3 + j])

    def prefetch(b):
        v_copy(b + 1).start()
        q_copy(b + 2).start()
        k_copy(b + 2).start()

    def start_copies(b):
        @pl.when(b >= 1)
        def _():
            o_copy(b - 1, HB - 1).start()

        prefetch(b)

    def pack_lhs(ks):
        row = lax.broadcasted_iota(I32, (8, tk), 0)
        lane = lax.broadcasted_iota(I32, (8, KA), 1)
        e0 = jnp.where(row == 0, 1.0, 0.0)
        e01 = jnp.where(row < 2, 1.0, 0.0)
        aug = jnp.concatenate(
            [ks, e0, e0, ks * EPS, e01, jnp.zeros_like(e0)], axis=0).astype(BF16)
        z = pltpu.bitcast(aug.T, U32)
        out = []
        for i in range(ng // 2):
            hi_g, lo_g = ng - 1 - 2 * i, ng - 2 - 2 * i
            out.append(jnp.where(lane < lo0, z[8 * hi_g:8 * hi_g + 8],
                                 z[8 * lo_g:8 * lo_g + 8]))
        return out

    def prep_k(bn, j, ci, run):
        ks = kb_ref[bn & 3, j, :, pl.ds(ci * tk, tk)].astype(F32) * c
        zs = pack_lhs(ks)
        for i, zz in enumerate(zs):
            kt_refs[j][bn & 1, pl.ds(ci * 32 + 8 * i, 8), :] = zz
        n2 = jnp.sum(ks * ks, axis=0, keepdims=True)
        return (n2 if run is None else jnp.maximum(run, n2)), zs[0]

    def prep_q(bn, j, i, run):
        qb = qb_ref[bn & 1, j, :, i * 128:(i + 1) * 128]
        w_ref[bn & 1, j, :, i * 128:(i + 1) * 128] = pltpu.bitcast(qb, U32)
        x = qb.astype(F32)
        n2 = jnp.sum(x * x, axis=0, keepdims=True)
        return n2 if run is None else jnp.maximum(run, n2)

    def const_rows(p2):
        row = lax.broadcasted_iota(I32, (8, 128), 0)
        a0 = jnp.where(row == 0, 1.5 * 2.0 ** 12, 0.0) * p2
        b0 = jnp.where(row == 0, -1.5, jnp.where(row == 1, -(2.0 ** -12), 0.0)) * p2
        wa = jnp.concatenate([a0, -a0], axis=0).astype(BF16)
        wb = jnp.concatenate([b0, jnp.zeros_like(b0)], axis=0).astype(BF16)
        return pltpu.bitcast(wa, U32), pltpu.bitcast(wb, U32)

    def prep_scale(bn, j, rq, rk):
        mq = jnp.max(rq, axis=1, keepdims=True) + 2.0 ** -100
        mk = jnp.max(rk, axis=1, keepdims=True) + 2.0 ** -100
        b2 = jnp.broadcast_to(mq * mk, (8, 128))
        p2 = jnp.full((8, 128), 2.0 ** XMAX, F32)
        up = jnp.full((8, 128), 2.0 ** (2 ** XMAX), F32)
        for x in reversed(range(XMAX)):
            ok = b2 <= (MARGIN * 2.0 ** (x - 1)) ** 2
            p2 = jnp.where(ok, 2.0 ** x, p2)
            up = jnp.where(ok, 2.0 ** (2 ** x), up)
        fast = jnp.where(b2 <= (MARGIN * 2.0 ** (XMAX - 1)) ** 2, 1, 0).astype(I32)
        consts = const_rows(p2)
        up_ref[bn & 1, j] = up
        cw_ref[bn & 1, j, 0] = consts[0]
        cw_ref[bn & 1, j, 1] = consts[1]
        return consts, fast

    def packed_dot(kc, wq, consts):
        w = jnp.concatenate([wq, widen(consts[0]), wq, widen(consts[1])], axis=0)
        return jnp.dot(pltpu.bitcast(kc, BF16), pltpu.bitcast(w, BF16),
                       preferred_element_type=F32)

    def qk(slot, j, tile, ci, consts, ltie=None):
        n = 32 * CPS
        kc = kt_refs[j][slot, pl.ds(ci * n, n), :]
        if ltie is not None:
            kc = jnp.concatenate(
                [kc[0:n - 8], jnp.where(ltie[0], kc[n - 8:n], ltie[1])], axis=0)
        return packed_dot(kc, w_ref[slot, j, :, tile * tq:(tile + 1) * tq], consts)

    def decode(tt):
        hi = pltpu.bitcast(pltpu.bitcast(tt, U32) & jnp.uint32(0xFFFFF000), F32)
        return hi, (tt - hi) * (1.0 / EPS)

    def exp_chunk(tt, lh, ll):
        hi, lo = decode(tt)
        ph, plo = jnp.exp2(hi), jnp.exp2(lo)
        grp = [None] * (ng * CPS)
        for cc in range(CPS):
            for i in range(ng // 2):
                r0 = 64 * cc + 16 * i
                a = ph[r0:r0 + 8] + ph[r0 + 8:r0 + 16]
                b = plo[r0:r0 + 8] + plo[r0 + 8:r0 + 16]
                lh = a if lh is None else lh + a
                ll = b if ll is None else ll + b
                grp[cc * ng + ng - 1 - 2 * i] = ph[r0:r0 + 16]
                grp[cc * ng + ng - 2 - 2 * i] = plo[r0:r0 + 16]
        return jnp.concatenate(grp, axis=0).astype(BF16), lh, ll

    def store_carry(tt0):
        lh = ll = None
        for e in range(LEAD):
            p, lh, ll = exp_chunk(tt0[e], lh, ll)
            p0_ref[e] = p
        l0_ref[0] = lh
        l0_ref[1] = ll

    def full_prep(bn):
        allfast = None
        for j in range(HB):
            rq = rk = None
            for i in range(nc):
                rq = prep_q(bn, j, i, rq)
            for ci in range(nc):
                rk, _ = prep_k(bn, j, ci, rk)
            consts, fast = prep_scale(bn, j, rq, rk)
            if j == 0:
                store_carry([qk(bn & 1, 0, 0, e, consts) for e in range(LEAD)])
            allfast = fast if allfast is None else allfast * fast
        return allfast[0, 0]

    def probe():
        r = lax.broadcasted_iota(I32, (D, tk), 0)
        cc = lax.broadcasted_iota(I32, (D, tk), 1)
        ks = (((r * 37 + cc * 11) & 127) - 63).astype(F32) * (2.0 ** -9)
        r = lax.broadcasted_iota(I32, (D, tq), 0)
        cc = lax.broadcasted_iota(I32, (D, tq), 1)
        kc = jnp.concatenate(pack_lhs(ks) * CPS, axis=0)
        consts = const_rows(jnp.ones((8, 128), F32))
        err = None
        for rep in range(2):
            qs = (((r * 29 + cc * (13 + 4 * rep)) & 127) - 63).astype(F32) * (2.0 ** -10)
            qs = qs.astype(BF16)
            hi, lo = decode(packed_dot(kc, pltpu.bitcast(qs, U32), consts))
            ex = lax.dot_general(ks.astype(BF16), qs, (((0,), (0,)), ((), ())),
                                 preferred_element_type=F32)
            for i in range(CPS * ng // 2):
                hi_g, lo_g = ng - 1 - 2 * (i % 4), ng - 2 - 2 * (i % 4)
                e1 = jnp.abs(hi[16 * i:16 * i + 16] + 1.5 - ex[16 * hi_g:16 * hi_g + 16])
                e2 = jnp.abs(lo[16 * i:16 * i + 16] + 0.5 - ex[16 * lo_g:16 * lo_g + 16])
                e = jnp.maximum(e1, e2)
                err = e if err is None else jnp.maximum(err, e)
        bad = jnp.where(err <= 2.0 ** -11, 0.0, 1.0)
        return jnp.where(jnp.max(bad) == 0.0, 1, 0).astype(I32)

    def exact_block(b):
        start_copies(b)
        cur = b & 1
        tq, nq = TQE, S // TQE
        n_tiles = HB * nq
        always = widen(up_ref[cur, 0], tq) > 0.0
        for j in range(HB):
            for ci in range(nc):
                kr_ref[j, pl.ds(ci * 64, 64), :] = pltpu.bitcast(
                    kb_ref[b & 3, j, :, pl.ds(ci * tk, tk)].T, U32)

        def stage(it_qk, it_pv, m):
            if it_qk is not None:
                jq = it_qk // nq
                qoff = pl.multiple_of((it_qk % nq) * tq, tq)
                wq = pltpu.bitcast(w_ref[cur, jq, :, pl.ds(qoff, tq)], BF16)
            if it_pv is not None:
                jv = it_pv // nq
            m8 = l8 = acc = prev = None
            for ci in range(nc):
                if it_pv is not None:
                    s_cur = s_ref[pl.ds(ci * tk, tk), :]
                cm = None
                if it_qk is not None:
                    kc = pltpu.bitcast(kr_ref[jq, pl.ds(ci * 64, 64), :], BF16)
                    s = jnp.dot(kc, wq, preferred_element_type=F32)
                    s_ref[pl.ds(ci * tk, tk), :] = s
                    cm = [jnp.maximum(s[16 * r:16 * r + 8], s[16 * r + 8:16 * r + 16])
                          for r in range(ng)]
                    for a in cm:
                        m8 = a if m8 is None else jnp.maximum(m8, a)
                if it_pv is not None:
                    ps = [None] * ng
                    for i, r in enumerate(reversed(range(ng))):
                        if i % 2 == 0:
                            mg = m if prev is None else jnp.where(always, m, prev[i])
                        pa = jnp.exp2((s_cur[16 * r:16 * r + 8] - mg) * c)
                        pb = jnp.exp2((s_cur[16 * r + 8:16 * r + 16] - mg) * c)
                        l8 = pa + pb if l8 is None else l8 + (pa + pb)
                        ps[r] = jnp.concatenate([pa, pb], axis=0)
                    p = jnp.concatenate(ps, axis=0).astype(BF16)
                    pv = jnp.dot(vb_ref[cur, jv, :, pl.ds(ci * tk, tk)], p,
                                 preferred_element_type=F32)
                    acc = pv if acc is None else pv + acc
                prev = cm
            if it_pv is not None:
                l = jnp.sum(l8, axis=0, keepdims=True)
                off = pl.multiple_of((it_pv % nq) * tq, tq)
                ob_ref[cur, jv, :, pl.ds(off, tq)] = (acc * (1.0 / l)).astype(ob_ref.dtype)
            if it_qk is None:
                return None
            return jnp.broadcast_to(jnp.max(m8, axis=0, keepdims=True), (8, tq))

        m = stage(0, None, None)
        nfast = full_prep(b + 1)
        m = lax.fori_loop(0, n_tiles - 1, lambda i, mm: stage(i + 1, i, mm), m)
        for j in range(HB - 1):
            o_copy(b, j).start()
        stage(None, n_tiles - 1, m)
        return nfast

    def packed_block(b):
        cur = b & 1
        bn = b + 1
        consts = [(cw_ref[cur, j, 0], cw_ref[cur, j, 1]) for j in range(HB)]
        ups = [up_ref[cur, j] for j in range(HB)]
        lane = lax.broadcasted_iota(I32, (8, tk), 1)
        odd = (lane // 16) % 2 == 1

        always = ups[0] > 0.0
        ties, lties = {}, {}

        def tie(e, val):
            if val.dtype != U32:
                val = pltpu.bitcast(jnp.broadcast_to(val, (8, 128)), U32)
            ties.setdefault(e, []).append(val)

        def prep_v(j, ci, e_tie):
            upv = jnp.where(odd, ups[j], 1.0)
            vf = vb_ref[cur, j, :, pl.ds(ci * tk, tk)].astype(F32)
            vf = (vf.reshape(D // 8, 8, tk) * upv[None]).reshape(D, tk)
            vhu = pltpu.bitcast(vf.astype(BF16), U32)
            vh_ref[cur, j, :, pl.ds(ci * tk, tk)] = vhu
            if e_tie is not None:
                tie(e_tie, vhu[0:8])
                tie(e_tie, vhu[8:16])

        ns = nc // CPS
        per_head = nq * ns
        n_steps = HB * per_head
        tts, tt0, runs = {}, [], []
        lh = ll = acc = rq = rk = allfast = nconsts0 = None
        for e in range(n_steps):
            j, el = divmod(e, per_head)
            tile, ci = divmod(el, ns)
            if e + LEAD < n_steps:
                j1, el1 = divmod(e + LEAD, per_head)
                t1, c1 = divmod(el1, ns)
                cb = consts[j1][1]
                vals = ties.pop(e + 2, [])
                if vals:
                    cb = jnp.where(always, cb, functools.reduce(jnp.bitwise_or, vals))
                vals = lties.pop(e + 2, [])
                lt = (always[:, :KA], functools.reduce(jnp.bitwise_or, vals)) if vals else None
                tts[e + LEAD] = qk(cur, j1, t1, c1, (consts[j1][0], cb), lt)
            else:
                tt0.append(qk(bn & 1, 0, 0, e + LEAD - n_steps, nconsts0))
            if e == 0:
                start_copies(b)
                for cv in range(nc):
                    prep_v(0, cv, None)
            if j >= 1 and el == 8:
                o_copy(b, j - 1).start()
            jp = (j + 1) % HB
            if el == 0:
                rq = rk = None
            if (el - Q0) % QSTEP == 0 and 0 <= (el - Q0) // QSTEP < nc:
                rq = prep_q(bn, jp, (el - Q0) // QSTEP, rq)
                tie(e + TIE_LAG, rq)
            if (el - K0) % KSTEP == 0 and 0 <= (el - K0) // KSTEP < nc:
                rk, z0 = prep_k(bn, jp, (el - K0) // KSTEP, rk)
                tie(e + TIE_LAG, rk)
                if j < HB - 1:
                    lties.setdefault(j * per_head + Z_AT, []).append(z0)
            if j + 1 < HB and (el - V0) % VSTEP == 0 and 0 <= (el - V0) // VSTEP < nc:
                prep_v(j + 1, (el - V0) // VSTEP, e + TIE_LAG)
            if el == FIN:
                runs.append((jp, rq, rk))
                if j == HB - 1:
                    for jn, rqn, rkn in runs:
                        nconsts, fast = prep_scale(bn, jn, rqn, rkn)
                        tie(e + TIE_LAG, nconsts[0])
                        tie(e + TIE_LAG, nconsts[1])
                        if jn == 0:
                            nconsts0 = nconsts
                        allfast = fast if allfast is None else allfast * fast
            if ci == 0:
                lh = ll = None
            if e == 0:
                lh, ll = l0_ref[0], l0_ref[1]
            if e < LEAD:
                p = p0_ref[e]
            else:
                p, lh, ll = exp_chunk(tts.pop(e), lh, ll)
            vh = pltpu.bitcast(vh_ref[cur, j, :, pl.ds(ci * tk * CPS, tk * CPS)], BF16)
            pv = jnp.dot(vh, p, preferred_element_type=F32)
            acc = pv if ci == 0 else pv + acc
            if ci == ns - 1:
                l = jnp.sum(lh * widen(ups[j]) + ll, axis=0, keepdims=True)
                r0 = pl.reciprocal(l, approx=True)
                rinv = r0 * (2.0 - l * r0)
                ob_ref[cur, j, :, tile * tq:(tile + 1) * tq] = (acc * rinv).astype(ob_ref.dtype)
        store_carry(tt0)
        return allfast[0, 0]

    zero = jnp.int32(0)
    q0_copy = pltpu.make_async_copy(q_hbm.at[0], qb_ref.at[0], sem.at[3])
    k0_copy = pltpu.make_async_copy(k_hbm.at[0], kb_ref.at[0], sem.at[4])
    q0_copy.start()
    k0_copy.start()
    prefetch(zero - 1)
    ok = probe()
    q0_copy.wait()
    k0_copy.wait()
    fast0 = full_prep(zero) * ok

    def sync(b):
        v_copy(b).wait()
        q_copy(b + 1).wait()
        k_copy(b + 1).wait()

        @pl.when(b >= 1)
        def _():
            for j in range(HB - 1):
                o_copy(b - 1, j).wait()

        @pl.when(b >= 2)
        def _():
            o_copy(b - 2, HB - 1).wait()

    def body(b, fast):
        sync(b)
        return lax.cond(fast == 1, packed_block, exact_block, b) * ok

    lax.fori_loop(0, NB, body, fast0)
    last = jnp.int32(NB)
    sync(last)
    o_copy(last - 1, HB - 1).start()
    o_copy(last - 1, HB - 1).wait()


@jax.jit
def pallas_standalone__fused_io_aware_attn__prompt_kernel(
    q: jax.Array,
    k: jax.Array,
    v: jax.Array,
):
    B, H, S, D = q.shape
    NB = B * H // HB
    qT, kT, vT = (jnp.swapaxes(x, -1, -2).reshape(NB, HB, D, S) for x in (q, k, v))
    hbm = pl.BlockSpec(memory_space=pl.ANY)
    oT = pl.pallas_call(
        _attn_kernel,
        in_specs=[hbm, hbm, hbm],
        out_specs=hbm,
        out_shape=jax.ShapeDtypeStruct((NB, HB, D, S), q.dtype),
        scratch_shapes=[
            pltpu.VMEM((2, HB, D, S), BF16),
            pltpu.VMEM((4, HB, D, S), BF16),
            pltpu.VMEM((2, HB, D, S), BF16),
            pltpu.VMEM((2, HB, D, S), BF16),
            pltpu.SemaphoreType.DMA((3 + HB,)),
            pltpu.VMEM((2, HB, D // 2, S), U32),
            pltpu.VMEM((2, HB, D // 2, S), U32),
            pltpu.VMEM((LEAD, TK * CPS, TQ), BF16),
            pltpu.VMEM((2, 8, TQ), F32),
            pltpu.VMEM((2, HB, 8, 128), F32),
            pltpu.VMEM((2, HB, 2, 8, 128), U32),
            pltpu.VMEM((S, TQE), F32),
            pltpu.VMEM((HB, S // 2, D), U32),
        ] + [pltpu.VMEM((2, S // 4, KA), U32)] * HB,
        compiler_params=pltpu.CompilerParams(
            disable_bounds_checks=True,
            vmem_limit_bytes=64 * 1024 * 1024),
    )(qT, kT, vT)
    return jnp.swapaxes(oT.reshape(B, H, D, S), -1, -2)
```
